```python
import jax
import jax.numpy as jnp

def _softmax(x, axis=-1):
    return jax.nn.softmax(x, axis=axis)
def _gelu(x):
    return jax.nn.gelu(x, approximate=True)
def _silu(x):
    return jax.nn.silu(x)
def _sigmoid(x):
    return jax.nn.sigmoid(x)
def _layernorm(x, axis=-1, eps=1e-5):
    m = jnp.mean(x, axis=axis, keepdims=True)
    v = jnp.var(x, axis=axis, keepdims=True)
    return (x - m) / jnp.sqrt(v + eps)
def _scatter_add(tgt, idx, src, axis=0):
    return tgt.at[idx].add(src)
def _segment_sum(src, seg, n):
    return jax.ops.segment_sum(src, seg, n)
class _Rng:
    def __init__(self, key):
        self._k = key
    def _next(self):
        self._k, sub = jax.random.split(self._k)
        return sub
    def normal(self, shape):
        return jax.random.normal(self._next(), shape, dtype=jnp.bfloat16)
    def randint(self, lo, hi, shape):
        return jax.random.randint(self._next(), shape, lo, hi, dtype=jnp.int32)
    def uniform(self, shape, lo=0.0, hi=1.0):
        return jax.random.uniform(self._next(), shape, jnp.bfloat16, lo, hi)
    def permutation(self, n):
        return jax.random.permutation(self._next(), n)


kernel_name = 'interleave_layers__sliding_block_cached__mixer_s_mlp__decode'

def setup_inputs():
    _rng = _Rng(jax.random.key(int.from_bytes(__import__("os").urandom(4), "little")))
    _w = (lambda a: (lambda t: t.astype(jnp.bfloat16) if jnp.issubdtype(t.dtype, jnp.floating) else t)(jnp.asarray(a)))
    def _A_setup():
        B, Sq, D = 1, 1, 640
        Hq, Hkv, Sk, Dh = 32, 32, 32768, 192
        assert Hq % Hkv == 0, (Hq, Hkv)
        return {
            "x": _w((lambda *s: _rng.normal(s) * 0.05)(B, Sq, D)),
            "k_cache": _w((lambda *s: _rng.normal(s) * 0.05)(B, Hkv, Sk, Dh)),
            "v_cache": _w((lambda *s: _rng.normal(s) * 0.05)(B, Hkv, Sk, Dh)),
            "wq": _w((lambda *s: _rng.normal(s) * 0.05)(D, Hq * Dh) * (D ** -0.5)),
            "wo": _w((lambda *s: _rng.normal(s) * 0.05)(Hq * Dh, D) * ((Hq * Dh) ** -0.5)),
        }
    _A_in = _A_setup()

    def _B_setup():
        B, S, D, F = 1, 1, 640, 1536
        return {
            "x":  _w((lambda *s: _rng.normal(s) * 0.05)(B, S, D)),
            "w1": _w((lambda *s: _rng.normal(s) * 0.05)(D, D) * (D ** -0.5)),
            "w2": _w((lambda *s: _rng.normal(s) * 0.05)(D, D) * (D ** -0.5)),
            "w3": _w((lambda *s: _rng.normal(s) * 0.05)(D, F) * (D ** -0.5)),
            "w4": _w((lambda *s: _rng.normal(s) * 0.05)(F, D) * (F ** -0.5)),
        }
    _B_in = _B_setup()

    return {
        "A_x": _A_in["x"],
        "A_k_cache": _A_in["k_cache"],
        "A_v_cache": _A_in["v_cache"],
        "A_wq": _A_in["wq"],
        "A_wo": _A_in["wo"],
        "B_x": _B_in["x"],
        "B_w1": _B_in["w1"],
        "B_w2": _B_in["w2"],
        "B_w3": _B_in["w3"],
        "B_w4": _B_in["w4"],
    }

def reference(A_x, A_k_cache, A_v_cache, A_wq, A_wo, B_x, B_w1, B_w2, B_w3, B_w4):
    def _A_ref(x, k_cache, v_cache, wq, wo):
        B, Sq, D = x.shape
        Hq, Dh = 32, 192
        Hkv, Sk = k_cache.shape[1], k_cache.shape[2]
        W = min(4096, max(256, Sk // 4))
        rep = Hq // Hkv
        q = (lambda x, *d: x.transpose(*d))((x @ wq).reshape(B, Sq, Hq, Dh), 0, 2, 1, 3)
        k = jnp.repeat(k_cache[:, :, Sk - W:, :], rep, axis=1)
        v = jnp.repeat(v_cache[:, :, Sk - W:, :], rep, axis=1)
        scores = jnp.einsum("bhqd,bhkd->bhqk", q, k) * (Dh ** -0.5)
        p = _softmax(scores, axis=-1)
        o = jnp.einsum("bhqk,bhkd->bhqd", p, v)
        return (lambda x, *d: x.transpose(*d))(o, 0, 2, 1, 3).reshape(B, Sq, Hq * Dh) @ wo

    def _B_ref(x, w1, w2, w3, w4):
        B, S, D = x.shape
        h = _gelu(_layernorm(x, axis=-1) @ w1)
        c = D // 4
        g0 = jnp.pad(h[:, :, 0*c:1*c], ((0, 0), (1, 0), (0, 0)))[:, :S, :]
        g1 = jnp.pad(h[:, :, 1*c:2*c], ((0, 0), (0, 1), (0, 0)))[:, 1:, :]
        g2 = jnp.pad(h[:, :, 2*c:3*c], ((0, 0), (2, 0), (0, 0)))[:, :S, :]
        g3 = jnp.pad(h[:, :, 3*c:   ], ((0, 0), (0, 2), (0, 0)))[:, 2:, :]
        hs = jnp.concatenate([g0, g1, g2, g3], axis=-1) @ w2
        x1 = x + hs
        h2 = _gelu(_layernorm(x1, axis=-1) @ w3) @ w4
        return x1 + h2

    x = A_x
    x = x + _A_ref(_layernorm(x, axis=-1), A_k_cache, A_v_cache, A_wq, A_wo)
    x = x + _B_ref(_layernorm(x, axis=-1), B_w1, B_w2, B_w3, B_w4)
    x = x + _A_ref(_layernorm(x, axis=-1), A_k_cache, A_v_cache, A_wq, A_wo)
    x = x + _B_ref(_layernorm(x, axis=-1), B_w1, B_w2, B_w3, B_w4)
    return x
```

```python
import jax
import jax.numpy as jnp
import jax.experimental.pallas as pl
import jax.experimental.pallas.tpu as pltpu

H, DH, D, F = 32, 192, 640, 1536
HD = H * DH
G = 8
NG = H // G
GR = G * DH
LANE = 128
EPS = 1e-5


def _ln(x):
    m = jnp.mean(x, axis=-1, keepdims=True)
    xc = x - m
    v = jnp.mean(xc * xc, axis=-1, keepdims=True)
    return xc * jax.lax.rsqrt(v + EPS)


def _gelu(x):
    c = 0.7978845608028654
    return 0.5 * x * (1.0 + jnp.tanh(c * (x + 0.044715 * (x * x * x))))


def _bf(w):
    return pltpu.bitcast(w, jnp.bfloat16)


def _dot(a, b):
    return jnp.dot(a, b, preferred_element_type=jnp.float32)


def _dot_nt(a, b):
    return jax.lax.dot_general(a, b, (((1,), (1,)), ((), ())),
                               preferred_element_type=jnp.float32)


def _make_kernel(sk, w):
    ns = w // LANE
    s0 = sk - w
    scale = DH ** -0.5

    def kernel(x_hbm, k_hbm, v_hbm, wq_hbm, wo_hbm, w3_hbm, w4_hbm, o_ref,
               xb, kb, vb, wqb, wob, w3b, w4b, qb, sb, mb, ob, lb, sems):
        kw = kb.bitcast(jnp.int32)
        vw = vb.bitcast(jnp.int32)
        wqw = wqb.bitcast(jnp.int32)
        wow = wob.bitcast(jnp.int32)
        w3w = w3b.bitcast(jnp.int32)
        w4w = w4b.bitcast(jnp.int32)

        SX, SWQ, SWO, SW3, SW4, SK0, SV0 = 0, 1, 2, 3, 4, 5, 5 + NG

        def start_w(src, dst, sem):
            for n in range(dst.shape[0]):
                pltpu.make_async_copy(src.at[:, n * LANE:(n + 1) * LANE],
                                      dst.at[n], sems.at[sem]).start()

        def wait_all(dst, sem):
            pltpu.make_async_copy(dst, dst, sems.at[sem]).wait()

        def start_kv(src, dst, g, sem):
            r0 = pl.multiple_of(g * GR, GR)
            for c in range(ns):
                pltpu.make_async_copy(
                    src.at[pl.ds(r0, GR), pl.ds(s0 + c * LANE, LANE)],
                    dst.at[c, pl.ds(r0, GR), :], sems.at[sem]).start()

        def wait_kv(dst, g, sem):
            r0 = pl.multiple_of(g * GR, GR)
            d = dst.at[:, pl.ds(r0, GR), :]
            pltpu.make_async_copy(d, d, sems.at[sem]).wait()

        pltpu.make_async_copy(x_hbm, xb, sems.at[SX]).start()
        start_w(wq_hbm, wqb, SWQ)
        start_kv(k_hbm, kb, 0, SK0)
        pltpu.make_async_copy(x_hbm, xb, sems.at[SX]).wait()
        x0 = xb[...].astype(jnp.float32)

        row = jax.lax.broadcasted_iota(jnp.int32, (G, LANE), 0)
        lane = jax.lax.broadcasted_iota(jnp.int32, (G, LANE), 1)

        def head_mask(t):
            j, r = divmod(t, 3)
            if r == 0:
                return row == 2 * j
            if r == 2:
                return row == 2 * j + 1
            return row == jnp.where(lane >= 64, 2 * j + 1, 2 * j)

        masks = [head_mask(t) for t in range(GR // LANE)]

        def layer(l, x):
            first = l == 0
            xn = _ln(x)
            xn8 = jnp.broadcast_to(xn, (G, D)).astype(jnp.bfloat16)

            @pl.when(first)
            def _():
                wait_all(wqb, SWQ)
                start_kv(k_hbm, kb, 1, SK0 + 1)

            for g in range(NG):
                for t in range(GR // LANE):
                    n = g * (GR // LANE) + t
                    q = _dot(xn8, _bf(wqw[n])) * scale
                    qb[g, :, t * LANE:(t + 1) * LANE] = jnp.where(
                        masks[t], q, 0.0).astype(jnp.bfloat16)

            def qk_group(g, _):
                @pl.when(first)
                def _():
                    wait_kv(kb, g, SK0 + g)

                    @pl.when(g + 2 < NG)
                    def _():
                        start_kv(k_hbm, kb, g + 2, SK0 + g + 2)

                    @pl.when(g + 2 >= NG)
                    def _():
                        start_kv(v_hbm, vb, g + 2 - NG, SV0 + g + 2 - NG)

                rw = pl.multiple_of(g * (GR // 2), GR // 2)
                qg = qb[g]
                mx = None
                for c in range(ns):
                    s = _dot(qg, _bf(kw[c, pl.ds(rw, GR // 2), :]))
                    sb[g, c] = s
                    mx = s if mx is None else jnp.maximum(mx, s)
                mb[g] = mx
                return 0

            jax.lax.fori_loop(0, NG, qk_group, 0)
            for g in range(NG):
                mb[g] = jnp.broadcast_to(
                    jnp.max(mb[g], axis=1, keepdims=True), (G, LANE))

            def pv_group(g, _):
                @pl.when(first)
                def _():
                    @pl.when(g == 0)
                    def _():
                        start_w(wo_hbm, wob, SWO)

                    wait_kv(vb, g, SV0 + g)

                    @pl.when(g + 2 < NG)
                    def _():
                        start_kv(v_hbm, vb, g + 2, SV0 + g + 2)

                    @pl.when(g + 2 == NG)
                    def _():
                        start_w(w3_hbm, w3b, SW3)
                        start_w(w4_hbm, w4b, SW4)

                rw = pl.multiple_of(g * (GR // 2), GR // 2)
                m = mb[g]
                lsum = None
                acc = None
                for c in range(ns):
                    p = jnp.exp(sb[g, c] - m)
                    lsum = p if lsum is None else lsum + p
                    r = _dot_nt(p.astype(jnp.bfloat16),
                                _bf(vw[c, pl.ds(rw, GR // 2), :]))
                    acc = r if acc is None else acc + r
                ob[g] = acc
                lb[g] = lsum
                return 0

            jax.lax.fori_loop(0, NG, pv_group, 0)

            @pl.when(first)
            def _():
                wait_all(wob, SWO)

            ys = [None] * (D // LANE)
            for g in range(NG):
                inv = 1.0 / jnp.sum(lb[g], axis=1, keepdims=True)
                og = jnp.concatenate(
                    [jnp.where(masks[t], ob[g, :, t * LANE:(t + 1) * LANE] * inv, 0.0)
                     for t in range(GR // LANE)], axis=1).astype(jnp.bfloat16)
                for n in range(D // LANE):
                    r = _dot(og, _bf(wow[n, g * (GR // 2):(g + 1) * (GR // 2), :]))
                    ys[n] = r if ys[n] is None else ys[n] + r
            attn = jnp.concatenate(
                [jnp.sum(y, axis=0, keepdims=True) for y in ys], axis=1)
            x = x + attn

            x1 = _ln(x)
            hn = jnp.broadcast_to(_ln(x1), (G, D)).astype(jnp.bfloat16)

            @pl.when(first)
            def _():
                wait_all(w3b, SW3)

            h = jnp.concatenate(
                [_gelu(_dot(hn, _bf(w3w[n]))) for n in range(F // LANE)],
                axis=1).astype(jnp.bfloat16)

            @pl.when(first)
            def _():
                wait_all(w4b, SW4)

            h2 = jnp.concatenate(
                [_dot(h, _bf(w4w[n])) for n in range(D // LANE)], axis=1)
            return x + x1 + h2[0:1, :]

        xf = jax.lax.fori_loop(0, 2, layer, x0)
        o_ref[...] = xf.astype(o_ref.dtype)

    return kernel


@jax.jit
def pallas_interleave_layers__sliding_block_cached__mixer_s_mlp__decode_kernel(
    A_x: jax.Array,
    A_k_cache: jax.Array,
    A_v_cache: jax.Array,
    A_wq: jax.Array,
    A_wo: jax.Array,
    B_x: jax.Array,
    B_w1: jax.Array,
    B_w2: jax.Array,
    B_w3: jax.Array,
    B_w4: jax.Array,
):
    del B_x, B_w1, B_w2
    sk = A_k_cache.shape[2]
    w = min(4096, max(256, sk // 4))
    ns = w // LANE
    k_t = jnp.transpose(A_k_cache, (0, 1, 3, 2)).reshape(HD, sk)
    v_t = jnp.transpose(A_v_cache, (0, 1, 3, 2)).reshape(HD, sk)
    x2 = A_x.reshape(1, D)

    any_spec = pl.BlockSpec(memory_space=pl.ANY)
    out = pl.pallas_call(
        _make_kernel(sk, w),
        in_specs=[any_spec] * 7,
        out_specs=pl.BlockSpec(memory_space=pltpu.VMEM),
        out_shape=jax.ShapeDtypeStruct((1, D), A_x.dtype),
        scratch_shapes=[
            pltpu.VMEM((1, D), jnp.bfloat16),
            pltpu.VMEM((ns, HD, LANE), jnp.bfloat16),
            pltpu.VMEM((ns, HD, LANE), jnp.bfloat16),
            pltpu.VMEM((HD // LANE, D, LANE), jnp.bfloat16),
            pltpu.VMEM((D // LANE, HD, LANE), jnp.bfloat16),
            pltpu.VMEM((F // LANE, D, LANE), jnp.bfloat16),
            pltpu.VMEM((D // LANE, F, LANE), jnp.bfloat16),
            pltpu.VMEM((NG, G, GR), jnp.bfloat16),
            pltpu.VMEM((NG, ns, G, LANE), jnp.float32),
            pltpu.VMEM((NG, G, LANE), jnp.float32),
            pltpu.VMEM((NG, G, GR), jnp.float32),
            pltpu.VMEM((NG, G, LANE), jnp.float32),
            pltpu.SemaphoreType.DMA((5 + 2 * NG,)),
        ],
        compiler_params=pltpu.CompilerParams(
            vmem_limit_bytes=128 * 1024 * 1024),
    )(x2, k_t, v_t, A_wq, A_wo, B_w3, B_w4)
    return out.reshape(A_x.shape)
```

```python
import jax
import jax.numpy as jnp
import jax.experimental.pallas as pl
import jax.experimental.pallas.tpu as pltpu

H, DH, D, F = 32, 192, 640, 1536
HD = H * DH
G = 8
NG = H // G
GR = G * DH
LANE = 128
NT = GR // LANE
EPS = 1e-5

NV = 12
NM = H - NV
MT = NM * DH // LANE
SBQ = 16
SBV = 16
TRB = 3


def _gelu(x):
    c = 0.7978845608028654
    return 0.5 * x * (1.0 + jnp.tanh(c * (x + 0.044715 * (x * x * x))))


def _bf(w):
    return pltpu.bitcast(w, jnp.bfloat16)


def _words(x8):
    x16 = jnp.concatenate([x8, jnp.zeros_like(x8)], axis=0).astype(jnp.bfloat16)
    return pltpu.bitcast(x16, jnp.int32)


def _dot(a, b):
    return jnp.dot(a, b, preferred_element_type=jnp.float32)


def _dot_nt(a, b):
    return jax.lax.dot_general(a, b, (((1,), (1,)), ((), ())),
                               preferred_element_type=jnp.float32)


def _interleave(tasks_m, tasks_v):
    nm, nv = len(tasks_m), len(tasks_v)
    im = 0
    for iv in range(nv):
        while im < nm and im * nv <= iv * nm:
            tasks_m[im]()
            im += 1
        tasks_v[iv]()
    while im < nm:
        tasks_m[im]()
        im += 1


def _make_kernel(sk, w):
    ns = w // LANE
    s0 = sk - w
    scale = DH ** -0.5

    def kernel(x_hbm, k_hbm, v_hbm, wq_hbm, wo_hbm, w3_hbm, w4_hbm, o_ref,
               xb, kb, vb, wqb, wob, w3b, w4b, qb, sa, sb, pb, qc, acc_b, part,
               ob, sems):
        kw = kb.bitcast(jnp.int32)
        vw = vb.bitcast(jnp.int32)
        wqw = wqb.bitcast(jnp.int32)
        wow = wob.bitcast(jnp.int32)
        w3w = w3b.bitcast(jnp.int32)
        w4w = w4b.bitcast(jnp.int32)

        SX, SWQ, SWO, SW3, SW4, SK0, SV0 = 0, 1, 2, 3, 4, 5, 5 + NG

        def start_w(src, dst, sem):
            for n in range(dst.shape[0]):
                pltpu.make_async_copy(src.at[:, n * LANE:(n + 1) * LANE],
                                      dst.at[n], sems.at[sem]).start()

        def wait_all(dst, sem):
            pltpu.make_async_copy(dst, dst, sems.at[sem]).wait()

        def start_kv(src, dst, g, sem):
            r0 = pl.multiple_of(g * GR, GR)
            for c in range(ns):
                pltpu.make_async_copy(
                    src.at[pl.ds(r0, GR), pl.ds(s0 + c * LANE, LANE)],
                    dst.at[c, pl.ds(r0, GR), :], sems.at[sem]).start()

        def wait_kv(dst, g, sem):
            r0 = pl.multiple_of(g * GR, GR)
            d = dst.at[:, pl.ds(r0, GR), :]
            pltpu.make_async_copy(d, d, sems.at[sem]).wait()

        pltpu.make_async_copy(x_hbm, xb, sems.at[SX]).start()
        start_w(wq_hbm, wqb, SWQ)
        start_kv(k_hbm, kb, 0, SK0)
        pltpu.make_async_copy(x_hbm, xb, sems.at[SX]).wait()
        x0 = xb[...].astype(jnp.float32)

        row = jax.lax.broadcasted_iota(jnp.int32, (G, LANE), 0)
        lane = jax.lax.broadcasted_iota(jnp.int32, (G, LANE), 1)

        def head_mask(t):
            j, r = divmod(t, 3)
            if r == 0:
                return row == 2 * j
            if r == 2:
                return row == 2 * j + 1
            return row == jnp.where(lane >= 64, 2 * j + 1, 2 * j)

        masks = [head_mask(t) for t in range(NT)]

        def ln_stats(x):
            m = jnp.mean(x, axis=-1, keepdims=True)
            xc = x - m
            v = jnp.mean(xc * xc, axis=-1, keepdims=True)
            return xc, v

        def mixer(x, first):
            xc, v = ln_stats(x)
            r1 = jax.lax.rsqrt(v + EPS)
            x1 = xc * r1
            hn = x1 * jax.lax.rsqrt(v * r1 * r1 + EPS)
            hn = jnp.broadcast_to(hn, (G, D)).astype(jnp.bfloat16)
            if first:
                wait_all(w3b, SW3)
            h = jnp.concatenate(
                [_gelu(_dot(hn, _bf(w3w[n]))) for n in range(F // LANE)],
                axis=1).astype(jnp.bfloat16)
            if first:
                wait_all(w4b, SW4)
            h2 = jnp.concatenate(
                [_dot(h, _bf(w4w[n])) for n in range(D // LANE)], axis=1)
            return x + x1 + h2[0:1, :]

        def out_proj():
            ys = [None] * (D // LANE)
            for g in range(NG):
                og = _bf(ob[g])
                for n in range(D // LANE):
                    r = _dot(og, _bf(wow[n, g * (GR // 2):(g + 1) * (GR // 2), :]))[0:G]
                    ys[n] = r if ys[n] is None else ys[n] + r
            return jnp.concatenate(
                [jnp.sum(y, axis=0, keepdims=True) for y in ys], axis=1)

        def q_input(x):
            xc, v = ln_stats(x)
            xn = xc * jax.lax.rsqrt(v + EPS)
            return jnp.broadcast_to(xn, (G, D)).astype(jnp.bfloat16)

        def layer1(x):
            xn8 = q_input(x)
            wait_all(wqb, SWQ)
            start_kv(v_hbm, vb, 0, SV0)
            for g in range(NG):
                for t in range(NT):
                    q = _dot(xn8, _bf(wqw[g * NT + t])) * scale
                    qb[g, :, t * LANE:(t + 1) * LANE] = _words(jnp.where(masks[t], q, 0.0))

            def group(g, _):
                wait_kv(kb, g, SK0 + g)

                @pl.when(g + 1 < NG)
                def _():
                    start_kv(k_hbm, kb, g + 1, SK0 + g + 1)

                @pl.when(g + 1 == NG)
                def _():
                    start_w(wo_hbm, wob, SWO)

                rw = pl.multiple_of(g * (GR // 2), GR // 2)
                qg = _bf(qb[g])
                mx = None
                for c in range(ns):
                    s = _dot(qg, _bf(kw[c, pl.ds(rw, GR // 2), :]))[0:G]
                    sa[g, c] = s
                    mx = s if mx is None else jnp.maximum(mx, s)
                m = jnp.max(mx, axis=1, keepdims=True)

                wait_kv(vb, g, SV0 + g)

                @pl.when(g + 1 < NG)
                def _():
                    start_kv(v_hbm, vb, g + 1, SV0 + g + 1)

                @pl.when(g + 1 == NG)
                def _():
                    start_w(w3_hbm, w3b, SW3)
                    start_w(w4_hbm, w4b, SW4)

                lsum = None
                acc = None
                for c in range(ns):
                    p = jnp.exp(sa[g, c] - m)
                    lsum = p if lsum is None else lsum + p
                    r = _dot_nt(p.astype(jnp.bfloat16), _bf(vw[c, pl.ds(rw, GR // 2), :]))
                    acc = r if acc is None else acc + r
                inv = 1.0 / jnp.sum(lsum, axis=1, keepdims=True)
                for t in range(NT):
                    ob[g, :, t * LANE:(t + 1) * LANE] = _words(
                        jnp.where(masks[t], acc[:, t * LANE:(t + 1) * LANE] * inv, 0.0))

                nblk = jnp.clip(MT // TRB - g * (NT // TRB), 0, NT // TRB)

                def tr(i, _):
                    c = i // jnp.maximum(nblk, 1)
                    t0 = (i % jnp.maximum(nblk, 1)) * TRB
                    r0 = pl.multiple_of(g * (GR // 2) + t0 * (LANE // 2), LANE // 2)
                    blk = _bf(vw[c, pl.ds(r0, TRB * LANE // 2), :])
                    outs = [pltpu.bitcast(blk[t * LANE:(t + 1) * LANE, :].T, jnp.int32)
                            for t in range(TRB)]
                    vw[c, pl.ds(r0, TRB * LANE // 2), :] = jnp.concatenate(outs, axis=0)
                    return 0

                jax.lax.fori_loop(0, ns * nblk, tr, 0)
                return 0

            jax.lax.fori_loop(0, NG, group, 0)
            wait_all(wob, SWO)
            x = x + out_proj()
            return mixer(x, True)

        def layer2(x):
            xn8 = q_input(x)
            for n in range(MT, HD // LANE):
                q = _dot(xn8, _bf(wqw[n])) * scale
                j = n - MT
                qc[j * LANE:(j + 1) * LANE, :] = jnp.broadcast_to(q[0:1], (LANE, LANE)).T
            for n in range(MT):
                g, t = divmod(n, NT)
                q = _dot(xn8, _bf(wqw[n])) * scale
                qb[g, :, t * LANE:(t + 1) * LANE] = _words(jnp.where(masks[t], q, 0.0))
            acc_b[...] = jnp.zeros(acc_b.shape, jnp.float32)

            def qk_body(b, _):
                c0 = b * SBQ
                tasks_m, tasks_v = [], []
                for ci in range(SBQ):
                    for t0 in range(0, MT, NT):
                        def tm(ci=ci, t0=t0):
                            c = c0 + ci
                            g = t0 // NT
                            nt = min(NT, MT - t0)
                            q = _bf(qb[g])
                            kc = _bf(kw[c, t0 * 64:(t0 + nt) * 64, :])
                            for t in range(nt):
                                r = _dot(q[:, t * LANE:(t + 1) * LANE], kc[t * LANE:(t + 1) * LANE, :])
                                jj, kind = divmod(t, 3)
                                if kind == 0:
                                    sa[g, c, 2 * jj:2 * jj + 1, :] = r[2 * jj:2 * jj + 1, :]
                                elif kind == 2:
                                    sa[g, c, 2 * jj + 1:2 * jj + 2, :] = r[2 * jj + 1:2 * jj + 2, :]
                                else:
                                    sb[g, c, 2 * jj:2 * jj + 2, :] = r[2 * jj:2 * jj + 2, :]
                        tasks_m.append(tm)
                for hv in range(NV):
                    def tv(hv=hv):
                        h = NM + hv
                        qs = [qc[(hv * 24 + j) * 8:(hv * 24 + j + 1) * 8, :] for j in range(24)]
                        for ci in range(SBQ):
                            c = c0 + ci
                            blk = kw[c, h * 96:(h + 1) * 96, :]
                            a0 = a1 = None
                            for d in range(12):
                                xk = _bf(blk[d * 8:(d + 1) * 8, :]).astype(jnp.float32)
                                u = xk[0:8] * qs[2 * d]
                                v = xk[8:16] * qs[2 * d + 1]
                                a0 = u if a0 is None else a0 + u
                                a1 = v if a1 is None else a1 + v
                            sa[h // G, c, h % G:h % G + 1, :] = jnp.sum(a0 + a1, axis=0, keepdims=True)
                    tasks_v.append(tv)
                _interleave(tasks_m, tasks_v)
                return 0

            jax.lax.fori_loop(0, ns // SBQ, qk_body, 0)

            invs = []
            for g in range(NG):
                n_m = min(max(NM - g * G, 0), G)
                ss = []
                mx = None
                for c in range(ns):
                    s = sa[g, c]
                    if n_m:
                        s = s + sb[g, c]
                    ss.append(s)
                    mx = s if mx is None else jnp.maximum(mx, s)
                m = jnp.max(mx, axis=1, keepdims=True)
                lsum = None
                for c in range(ns):
                    e = jnp.exp(ss[c] - m)
                    lsum = e if lsum is None else lsum + e
                    if n_m:
                        pb[g, c] = _words(e)
                    if n_m < G:
                        sa[g, c] = e
                invs.append(1.0 / jnp.sum(lsum, axis=1, keepdims=True))

            def pv_body(b, _):
                c0 = b * SBV
                tasks_m, tasks_v = [], []
                for ci in range(SBV):
                    for t0 in range(0, MT, NT):
                        def tm(ci=ci, t0=t0):
                            c = c0 + ci
                            g = t0 // NT
                            nt = min(NT, MT - t0)
                            p = _bf(pb[g, c])
                            vc = _bf(vw[c, t0 * 64:(t0 + nt) * 64, :])
                            for t in range(nt):
                                part[c, t0 + t] = _dot(p, vc[t * LANE:(t + 1) * LANE, :])[0:G]
                        tasks_m.append(tm)
                for hv in range(NV):
                    def tv(hv=hv):
                        h = NM + hv
                        ps = [jnp.broadcast_to(sa[h // G, c0 + ci, h % G:h % G + 1, :], (G, LANE))
                              for ci in range(SBV)]
                        for d in range(12):
                            a0 = a1 = None
                            for ci in range(SBV):
                                xv = _bf(vw[c0 + ci, h * 96 + d * 8:h * 96 + d * 8 + 8, :]).astype(jnp.float32)
                                u = xv[0:8] * ps[ci]
                                v = xv[8:16] * ps[ci]
                                a0 = u if a0 is None else a0 + u
                                a1 = v if a1 is None else a1 + v
                            r = (hv * 24 + 2 * d) * 8
                            acc_b[r:r + 8, :] = acc_b[r:r + 8, :] + a0
                            acc_b[r + 8:r + 16, :] = acc_b[r + 8:r + 16, :] + a1
                    tasks_v.append(tv)
                _interleave(tasks_m, tasks_v)
                return 0

            jax.lax.fori_loop(0, ns // SBV, pv_body, 0)

            for n in range(MT):
                g, t = divmod(n, NT)
                tot = None
                for c in range(ns):
                    tot = part[c, n] if tot is None else tot + part[c, n]
                ob[g, :, t * LANE:(t + 1) * LANE] = _words(
                    jnp.where(masks[t], tot * invs[g], 0.0))
            for j in range(NV * DH // LANE):
                rows = []
                for i in range(16):
                    hq = NM + (j * 16 + i) // 24
                    inv = jnp.broadcast_to(invs[hq // G][hq % G:hq % G + 1, :], (G, LANE))
                    r = (j * 16 + i) * 8
                    rows.append(acc_b[r:r + 8, :] * inv)
                tt = jnp.concatenate(rows, axis=0).T
                o8 = tt[0:8]
                for i in range(1, 16):
                    o8 = o8 + tt[i * 8:(i + 1) * 8]
                g, t = divmod(MT + j, NT)
                ob[g, :, t * LANE:(t + 1) * LANE] = _words(o8)
            x = x + out_proj()
            return mixer(x, False)

        sb[...] = jnp.zeros(sb.shape, jnp.float32)
        xf = layer2(layer1(x0))
        o_ref[...] = xf.astype(o_ref.dtype)

    return kernel


@jax.jit
def pallas_interleave_layers__sliding_block_cached__mixer_s_mlp__decode_kernel(
    A_x: jax.Array,
    A_k_cache: jax.Array,
    A_v_cache: jax.Array,
    A_wq: jax.Array,
    A_wo: jax.Array,
    B_x: jax.Array,
    B_w1: jax.Array,
    B_w2: jax.Array,
    B_w3: jax.Array,
    B_w4: jax.Array,
):
    del B_x, B_w1, B_w2
    sk = A_k_cache.shape[2]
    w = min(4096, max(256, sk // 4))
    ns = w // LANE
    k_t = jnp.transpose(A_k_cache, (0, 1, 3, 2)).reshape(HD, sk)
    v_t = jnp.transpose(A_v_cache, (0, 1, 3, 2)).reshape(HD, sk)
    x2 = A_x.reshape(1, D)

    any_spec = pl.BlockSpec(memory_space=pl.ANY)
    out = pl.pallas_call(
        _make_kernel(sk, w),
        in_specs=[any_spec] * 7,
        out_specs=pl.BlockSpec(memory_space=pltpu.VMEM),
        out_shape=jax.ShapeDtypeStruct((1, D), A_x.dtype),
        scratch_shapes=[
            pltpu.VMEM((1, D), jnp.bfloat16),
            pltpu.VMEM((ns, HD, LANE), jnp.bfloat16),
            pltpu.VMEM((ns, HD, LANE), jnp.bfloat16),
            pltpu.VMEM((HD // LANE, D, LANE), jnp.bfloat16),
            pltpu.VMEM((D // LANE, HD, LANE), jnp.bfloat16),
            pltpu.VMEM((F // LANE, D, LANE), jnp.bfloat16),
            pltpu.VMEM((D // LANE, F, LANE), jnp.bfloat16),
            pltpu.VMEM((NG, G, GR), jnp.int32),
            pltpu.VMEM((NG, ns, G, LANE), jnp.float32),
            pltpu.VMEM((NG, ns, G, LANE), jnp.float32),
            pltpu.VMEM((NG, ns, G, LANE), jnp.int32),
            pltpu.VMEM((NV * DH, LANE), jnp.float32),
            pltpu.VMEM((NV * DH, LANE), jnp.float32),
            pltpu.VMEM((ns, MT, G, LANE), jnp.float32),
            pltpu.VMEM((NG, G, GR), jnp.int32),
            pltpu.SemaphoreType.DMA((5 + 2 * NG,)),
        ],
        compiler_params=pltpu.CompilerParams(
            vmem_limit_bytes=128 * 1024 * 1024),
    )(x2, k_t, v_t, A_wq, A_wo, B_w3, B_w4)
    return out.reshape(A_x.shape)
```

```python
import jax
import jax.numpy as jnp
import jax.experimental.pallas as pl
import jax.experimental.pallas.tpu as pltpu

H, DH, D, F = 32, 192, 640, 1536
HD = H * DH
G = 8
NG = H // G
GR = G * DH
LANE = 128
NT = GR // LANE
ND = D // LANE
EPS = 1e-5

NV = 12
NM = H - NV
MT = NM * DH // LANE
SB = 16
TRB = 3
W4C = 3
FR = F // W4C


def _gelu(x):
    c = 0.7978845608028654
    return 0.5 * x * (1.0 + jnp.tanh(c * (x + 0.044715 * (x * x * x))))


def _bf(w):
    return pltpu.bitcast(w, jnp.bfloat16)


def _f32(w):
    x = _bf(w).astype(jnp.float32)
    return x[0:8], x[8:16]


def _words(x8):
    x16 = jnp.concatenate([x8, jnp.zeros_like(x8)], axis=0).astype(jnp.bfloat16)
    return pltpu.bitcast(x16, jnp.int32)


def _dot(a, b):
    return jnp.dot(a, b, preferred_element_type=jnp.float32)


def _dot_nt(a, b):
    return jax.lax.dot_general(a, b, (((1,), (1,)), ((), ())),
                               preferred_element_type=jnp.float32)


def _acc(a, b):
    return b if a is None else a + b


def _lanesum(a):
    return jnp.sum(a, axis=1, keepdims=True)


def _interleave(tasks_m, tasks_v):
    nm, nv = len(tasks_m), len(tasks_v)
    im = 0
    for iv in range(nv):
        while im < nm and im * nv <= iv * nm:
            tasks_m[im]()
            im += 1
        tasks_v[iv]()
    while im < nm:
        tasks_m[im]()
        im += 1


def _make_kernel(sk, w):
    ns = w // LANE
    s0 = sk - w
    sb_n = min(SB, ns)
    scale = DH ** -0.5

    def kernel(x_hbm, k_hbm, v_hbm, wq_hbm, wo_hbm, w3_hbm, w4_hbm, o_ref,
               xb, kb, vb, wqb, wob, w3b, w4b, qb, sa, sb, pb, qc, acc_b, part,
               ob, sems):
        kw = kb.bitcast(jnp.int32)
        vw = vb.bitcast(jnp.int32)
        wqw = wqb.bitcast(jnp.int32)
        wow = wob.bitcast(jnp.int32)
        w3w = w3b.bitcast(jnp.int32)
        w4w = w4b.bitcast(jnp.int32)

        SX, SWQ, SWO, SW3, SW4 = 0, 1, 2, 3, 4
        SK0 = SW4 + W4C
        SV0 = SK0 + NG

        def start_w(src, dst, sem):
            for n in range(dst.shape[0]):
                pltpu.make_async_copy(src.at[:, n * LANE:(n + 1) * LANE],
                                      dst.at[n], sems.at[sem]).start()

        def wait_all(dst, sem):
            pltpu.make_async_copy(dst, dst, sems.at[sem]).wait()

        def start_w4():
            for ch in range(W4C):
                for n in range(ND):
                    pltpu.make_async_copy(
                        w4_hbm.at[ch * FR:(ch + 1) * FR, n * LANE:(n + 1) * LANE],
                        w4b.at[n, ch * FR:(ch + 1) * FR, :],
                        sems.at[SW4 + ch]).start()

        def wait_w4(ch):
            wait_all(w4b.at[:, ch * FR:(ch + 1) * FR, :], SW4 + ch)

        def start_kv(src, dst, g, sem):
            r0 = pl.multiple_of(g * GR, GR)
            for c in range(ns):
                pltpu.make_async_copy(
                    src.at[pl.ds(r0, GR), pl.ds(s0 + c * LANE, LANE)],
                    dst.at[c, pl.ds(r0, GR), :], sems.at[sem]).start()

        def wait_kv(dst, g, sem):
            r0 = pl.multiple_of(g * GR, GR)
            wait_all(dst.at[:, pl.ds(r0, GR), :], sem)

        pltpu.make_async_copy(x_hbm, xb, sems.at[SX]).start()
        start_w(wq_hbm, wqb, SWQ)
        start_kv(k_hbm, kb, 0, SK0)
        wait_all(xb, SX)
        x0 = xb[...].astype(jnp.float32)

        row = jax.lax.broadcasted_iota(jnp.int32, (G, LANE), 0)
        lane = jax.lax.broadcasted_iota(jnp.int32, (G, LANE), 1)

        def head_mask(t):
            j, r = divmod(t, 3)
            if r == 0:
                return row == 2 * j
            if r == 2:
                return row == 2 * j + 1
            return row == jnp.where(lane >= 64, 2 * j + 1, 2 * j)

        masks = [head_mask(t) for t in range(NT)]

        def ln_stats(x):
            m = jnp.mean(x, axis=-1, keepdims=True)
            v = jnp.maximum(jnp.mean(x * x, axis=-1, keepdims=True) - m * m, 0.0)
            return x - m, v

        def mixer(x, streaming):
            xc, v = ln_stats(x)
            r1 = jax.lax.rsqrt(v + EPS)
            x1 = xc * r1
            hn = x1 * jax.lax.rsqrt(v * r1 * r1 + EPS)
            hn = jnp.broadcast_to(hn, (G, D)).astype(jnp.bfloat16)
            if streaming:
                wait_all(w3b, SW3)
            h = jnp.concatenate(
                [_gelu(_dot(hn, _bf(w3w[n]))) for n in range(F // LANE)],
                axis=1).astype(jnp.bfloat16)
            hs = [None] * ND
            for ch in range(W4C):
                if streaming:
                    wait_w4(ch)
                for n in range(ND):
                    hs[n] = _acc(hs[n], _dot(
                        h[:, ch * FR:(ch + 1) * FR],
                        _bf(w4w[n, ch * FR // 2:(ch + 1) * FR // 2, :])))
            return x + x1 + jnp.concatenate(hs, axis=1)[0:1, :]

        def q_store(g, t, q):
            qb[g, :, t * LANE:(t + 1) * LANE] = _words(jnp.where(masks[t], q, 0.0))

        def layer1(x):
            xc, v = ln_stats(x)
            xn8 = jnp.broadcast_to(xc * jax.lax.rsqrt(v + EPS),
                                   (G, D)).astype(jnp.bfloat16)
            wait_all(wqb, SWQ)
            start_kv(v_hbm, vb, 0, SV0)
            for n in range(HD // LANE):
                q_store(n // NT, n % NT, _dot(xn8, _bf(wqw[n])) * scale)

            def trq(n, _):
                blk = _bf(wqw[n])
                wqw[n] = jnp.concatenate(
                    [pltpu.bitcast(blk[kt * LANE:(kt + 1) * LANE, :].T, jnp.int32)
                     for kt in range(ND)], axis=0)
                return 0

            jax.lax.fori_loop(MT, HD // LANE, trq, 0)

            def group(g, _):
                wait_kv(kb, g, SK0 + g)

                @pl.when(g + 1 < NG)
                def _():
                    start_kv(k_hbm, kb, g + 1, SK0 + g + 1)

                @pl.when(g + 1 == NG)
                def _():
                    start_w(wo_hbm, wob, SWO)

                rw = pl.multiple_of(g * (GR // 2), GR // 2)
                qg = _bf(qb[g])
                mx = None
                for c in range(ns):
                    s = _dot(qg, _bf(kw[c, pl.ds(rw, GR // 2), :]))[0:G]
                    sa[g, c] = s
                    mx = s if mx is None else jnp.maximum(mx, s)
                m = jnp.max(mx, axis=1, keepdims=True)

                wait_kv(vb, g, SV0 + g)

                @pl.when(g + 1 < NG)
                def _():
                    start_kv(v_hbm, vb, g + 1, SV0 + g + 1)

                @pl.when(g + 1 == NG)
                def _():
                    start_w(w3_hbm, w3b, SW3)
                    start_w4()

                lsum = None
                acc = None
                for c in range(ns):
                    p = jnp.exp(sa[g, c] - m)
                    lsum = _acc(lsum, p)
                    acc = _acc(acc, _dot_nt(p.astype(jnp.bfloat16),
                                            _bf(vw[c, pl.ds(rw, GR // 2), :])))
                inv = 1.0 / _lanesum(lsum)
                for t in range(NT):
                    ob[g, :, t * LANE:(t + 1) * LANE] = _words(jnp.where(
                        masks[t], acc[:, t * LANE:(t + 1) * LANE] * inv, 0.0))

                def retile(t0, nt):
                    def tr(c, _):
                        r0 = pl.multiple_of(g * (GR // 2) + t0 * (LANE // 2), LANE // 2)
                        blk = _bf(vw[c, pl.ds(r0, nt * LANE // 2), :])
                        vw[c, pl.ds(r0, nt * LANE // 2), :] = jnp.concatenate(
                            [pltpu.bitcast(blk[t * LANE:(t + 1) * LANE, :].T, jnp.int32)
                             for t in range(nt)], axis=0)
                        return 0
                    jax.lax.fori_loop(0, ns, tr, 0)

                def blocks(i, _):
                    retile(i * TRB, TRB)
                    return 0

                nblk = jnp.clip(MT // TRB - g * (NT // TRB), 0, NT // TRB)
                jax.lax.fori_loop(0, nblk, blocks, 0)
                return 0

            jax.lax.fori_loop(0, NG, group, 0)
            wait_all(wob, SWO)
            ys = [None] * ND
            for g in range(NG):
                og = _bf(ob[g])
                for n in range(ND):
                    ys[n] = _acc(ys[n], _dot(
                        og, _bf(wow[n, g * (GR // 2):(g + 1) * (GR // 2), :]))[0:G])
            x = x + jnp.concatenate(
                [jnp.sum(y, axis=0, keepdims=True) for y in ys], axis=1)
            return mixer(x, True)

        def layer2(x):
            xc, v = ln_stats(x)
            xn = xc * jax.lax.rsqrt(v + EPS)
            xn8 = jnp.broadcast_to(xn, (G, D)).astype(jnp.bfloat16)

            xs = xn * scale
            xr = [jnp.broadcast_to(xs[:, kt * LANE:(kt + 1) * LANE], (G, LANE))
                  for kt in range(ND)]
            tasks_m, tasks_v = [], []
            for n in range(MT):
                def tm(n=n):
                    q_store(n // NT, n % NT, _dot(xn8, _bf(wqw[n])) * scale)
                tasks_m.append(tm)
            for n in range(MT, HD // LANE):
                for r in range(LANE // 16):
                    def tv(n=n, r=r):
                        a0 = a1 = None
                        for kt in range(ND):
                            w0, w1 = _f32(wqw[n, kt * 64 + r * 8:kt * 64 + r * 8 + 8, :])
                            a0 = _acc(a0, w0 * xr[kt])
                            a1 = _acc(a1, w1 * xr[kt])
                        r0 = (n - MT) * LANE + r * 16
                        qc[r0:r0 + 8, :] = jnp.broadcast_to(_lanesum(a0), (G, LANE))
                        qc[r0 + 8:r0 + 16, :] = jnp.broadcast_to(_lanesum(a1), (G, LANE))
                    tasks_v.append(tv)
            _interleave(tasks_m, tasks_v)
            acc_b[...] = jnp.zeros(acc_b.shape, jnp.float32)

            def qk_body(b, _):
                c0 = b * sb_n
                tasks_m, tasks_v = [], []
                for ci in range(sb_n):
                    for t0 in range(0, MT, NT):
                        def tm(ci=ci, t0=t0):
                            c = c0 + ci
                            g = t0 // NT
                            nt = min(NT, MT - t0)
                            q = _bf(qb[g])
                            kc = _bf(kw[c, t0 * 64:(t0 + nt) * 64, :])
                            for t in range(nt):
                                r = _dot(q[:, t * LANE:(t + 1) * LANE],
                                         kc[t * LANE:(t + 1) * LANE, :])
                                jj, kind = divmod(t, 3)
                                if kind == 0:
                                    sa[g, c, 2 * jj:2 * jj + 1, :] = r[2 * jj:2 * jj + 1, :]
                                elif kind == 2:
                                    sa[g, c, 2 * jj + 1:2 * jj + 2, :] = r[2 * jj + 1:2 * jj + 2, :]
                                else:
                                    sb[g, c, 2 * jj:2 * jj + 2, :] = r[2 * jj:2 * jj + 2, :]
                        tasks_m.append(tm)
                for hv in range(NV):
                    def tv(hv=hv):
                        h = NM + hv
                        qs = [qc[(hv * 24 + j) * 8:(hv * 24 + j + 1) * 8, :]
                              for j in range(24)]
                        for ci in range(sb_n):
                            c = c0 + ci
                            blk = kw[c, h * 96:(h + 1) * 96, :]
                            a0 = a1 = None
                            for d in range(12):
                                k0, k1 = _f32(blk[d * 8:(d + 1) * 8, :])
                                a0 = _acc(a0, k0 * qs[2 * d])
                                a1 = _acc(a1, k1 * qs[2 * d + 1])
                            sa[h // G, c, h % G:h % G + 1, :] = jnp.sum(
                                a0 + a1, axis=0, keepdims=True)
                    tasks_v.append(tv)
                _interleave(tasks_m, tasks_v)
                return 0

            jax.lax.fori_loop(0, ns // sb_n, qk_body, 0)

            invs = []
            for g in range(NG):
                n_m = min(max(NM - g * G, 0), G)
                ss = []
                mx = None
                for c in range(ns):
                    s = sa[g, c]
                    if n_m:
                        s = s + sb[g, c]
                    ss.append(s)
                    mx = s if mx is None else jnp.maximum(mx, s)
                m = jnp.max(mx, axis=1, keepdims=True)
                lsum = None
                for c in range(ns):
                    e = jnp.exp(ss[c] - m)
                    lsum = _acc(lsum, e)
                    if n_m:
                        pb[g, c] = _words(e)
                    if n_m < G:
                        sa[g, c] = e
                invs.append(1.0 / _lanesum(lsum))

            def pv_body(b, _):
                c0 = b * sb_n
                tasks_m, tasks_v = [], []
                for ci in range(sb_n):
                    for t0 in range(0, MT, NT):
                        def tm(ci=ci, t0=t0):
                            c = c0 + ci
                            g = t0 // NT
                            nt = min(NT, MT - t0)
                            p = _bf(pb[g, c])
                            vc = _bf(vw[c, t0 * 64:(t0 + nt) * 64, :])
                            for t in range(nt):
                                part[c, t0 + t] = _dot(
                                    p, vc[t * LANE:(t + 1) * LANE, :])[0:G]
                        tasks_m.append(tm)
                for hv in range(NV):
                    def tv(hv=hv):
                        h = NM + hv
                        ps = [jnp.broadcast_to(
                            sa[h // G, c0 + ci, h % G:h % G + 1, :], (G, LANE))
                            for ci in range(sb_n)]
                        for d in range(12):
                            a0 = a1 = None
                            for ci in range(sb_n):
                                v0, v1 = _f32(vw[c0 + ci,
                                                 h * 96 + d * 8:h * 96 + d * 8 + 8, :])
                                a0 = _acc(a0, v0 * ps[ci])
                                a1 = _acc(a1, v1 * ps[ci])
                            r = hv * DH + d * 16
                            acc_b[r:r + 8, :] = acc_b[r:r + 8, :] + a0
                            acc_b[r + 8:r + 16, :] = acc_b[r + 8:r + 16, :] + a1
                    tasks_v.append(tv)
                _interleave(tasks_m, tasks_v)
                return 0

            jax.lax.fori_loop(0, ns // sb_n, pv_body, 0)

            for n in range(MT):
                g, t = divmod(n, NT)
                tot = None
                for c in range(ns):
                    tot = _acc(tot, part[c, n])
                ob[g, :, t * LANE:(t + 1) * LANE] = _words(
                    jnp.where(masks[t], tot * invs[g], 0.0))

            ys = [None] * ND
            yv = [None] * ND
            tasks_m, tasks_v = [], []
            for kt in range(MT):
                def tm(kt=kt):
                    g, t = divmod(kt, NT)
                    og = _bf(ob[g, :, t * LANE:(t + 1) * LANE])
                    for n in range(ND):
                        ys[n] = _acc(ys[n], _dot(
                            og, _bf(wow[n, kt * 64:(kt + 1) * 64, :]))[0:G])
                tasks_m.append(tm)
            for hv in range(NV):
                def tv(hv=hv):
                    h = NM + hv
                    inv = jnp.broadcast_to(invs[h // G][h % G:h % G + 1, :], (G, LANE))
                    for d in range(12):
                        r = hv * DH + d * 16
                        o0 = _lanesum(acc_b[r:r + 8, :]) * inv
                        o1 = _lanesum(acc_b[r + 8:r + 16, :]) * inv
                        for n in range(ND):
                            w0, w1 = _f32(wow[n, h * 96 + d * 8:h * 96 + d * 8 + 8, :])
                            yv[n] = _acc(yv[n], w0 * o0 + w1 * o1)
                tasks_v.append(tv)
            _interleave(tasks_m, tasks_v)
            x = x + jnp.concatenate(
                [jnp.sum(a + b, axis=0, keepdims=True) for a, b in zip(ys, yv)],
                axis=1)
            return mixer(x, False)

        sb[...] = jnp.zeros(sb.shape, jnp.float32)
        o_ref[...] = layer2(layer1(x0)).astype(o_ref.dtype)

    return kernel


@jax.jit
def pallas_interleave_layers__sliding_block_cached__mixer_s_mlp__decode_kernel(
    A_x: jax.Array,
    A_k_cache: jax.Array,
    A_v_cache: jax.Array,
    A_wq: jax.Array,
    A_wo: jax.Array,
    B_x: jax.Array,
    B_w1: jax.Array,
    B_w2: jax.Array,
    B_w3: jax.Array,
    B_w4: jax.Array,
):
    del B_x, B_w1, B_w2
    sk = A_k_cache.shape[2]
    w = min(4096, max(256, sk // 4))
    ns = w // LANE
    k_t = jnp.transpose(A_k_cache, (0, 1, 3, 2)).reshape(HD, sk)
    v_t = jnp.transpose(A_v_cache, (0, 1, 3, 2)).reshape(HD, sk)
    x2 = A_x.reshape(1, D)

    any_spec = pl.BlockSpec(memory_space=pl.ANY)
    out = pl.pallas_call(
        _make_kernel(sk, w),
        in_specs=[any_spec] * 7,
        out_specs=pl.BlockSpec(memory_space=pltpu.VMEM),
        out_shape=jax.ShapeDtypeStruct((1, D), A_x.dtype),
        scratch_shapes=[
            pltpu.VMEM((1, D), jnp.bfloat16),
            pltpu.VMEM((ns, HD, LANE), jnp.bfloat16),
            pltpu.VMEM((ns, HD, LANE), jnp.bfloat16),
            pltpu.VMEM((HD // LANE, D, LANE), jnp.bfloat16),
            pltpu.VMEM((ND, HD, LANE), jnp.bfloat16),
            pltpu.VMEM((F // LANE, D, LANE), jnp.bfloat16),
            pltpu.VMEM((ND, F, LANE), jnp.bfloat16),
            pltpu.VMEM((NG, G, GR), jnp.int32),
            pltpu.VMEM((NG, ns, G, LANE), jnp.float32),
            pltpu.VMEM((NG, ns, G, LANE), jnp.float32),
            pltpu.VMEM((NG, ns, G, LANE), jnp.int32),
            pltpu.VMEM((NV * DH, LANE), jnp.float32),
            pltpu.VMEM((NV * DH, LANE), jnp.float32),
            pltpu.VMEM((ns, MT, G, LANE), jnp.float32),
            pltpu.VMEM((NG, G, GR), jnp.int32),
            pltpu.SemaphoreType.DMA((4 + W4C + 2 * NG,)),
        ],
        compiler_params=pltpu.CompilerParams(
            vmem_limit_bytes=128 * 1024 * 1024),
    )(x2, k_t, v_t, A_wq, A_wo, B_w3, B_w4)
    return out.reshape(A_x.shape)
```

```python
import jax
import jax.numpy as jnp
import jax.experimental.pallas as pl
import jax.experimental.pallas.tpu as pltpu

H, DH, D, F = 32, 192, 640, 1536
HD = H * DH
G = 8
NG = H // G
GR = G * DH
LANE = 128
NT = GR // LANE
ND = D // LANE
EPS = 1e-5

NV = 12
NM = H - NV
MT = NM * DH // LANE
SB = 16
TRB = 3
W4E = (0, 640, 1280, 1536)
W4C = len(W4E) - 1
WOC = 8


def _gelu(x):
    c = 0.7978845608028654
    return 0.5 * x * (1.0 + jnp.tanh(c * (x + 0.044715 * (x * x * x))))


def _bf(w):
    return pltpu.bitcast(w, jnp.bfloat16)


def _f32(w):
    x = _bf(w).astype(jnp.float32)
    return x[0:8], x[8:16]


def _words(x8):
    x16 = jnp.concatenate([x8, jnp.zeros_like(x8)], axis=0).astype(jnp.bfloat16)
    return pltpu.bitcast(x16, jnp.int32)


def _dot(a, b):
    return jnp.dot(a, b, preferred_element_type=jnp.float32)


def _dot_nt(a, b):
    return jax.lax.dot_general(a, b, (((1,), (1,)), ((), ())),
                               preferred_element_type=jnp.float32)


def _acc(a, b):
    return b if a is None else a + b


def _lanesum(a):
    return jnp.sum(a, axis=1, keepdims=True)


def _interleave(tasks_m, tasks_v):
    nm, nv = len(tasks_m), len(tasks_v)
    im = 0
    for iv in range(nv):
        while im < nm and im * nv <= iv * nm:
            tasks_m[im]()
            im += 1
        tasks_v[iv]()
    while im < nm:
        tasks_m[im]()
        im += 1


def _make_kernel(sk, w):
    ns = w // LANE
    s0 = sk - w
    sb_n = min(SB, ns)
    scale = DH ** -0.5

    def kernel(x_hbm, k_hbm, v_hbm, wq_hbm, wo_hbm, w3_hbm, w4_hbm, o_ref,
               xb, kb, vb, wqb, wob, w3b, w4b, qb, sa, sb, pb, qc, acc_b, part,
               ob, sems):
        kw = kb.bitcast(jnp.int32)
        vw = vb.bitcast(jnp.int32)
        wqw = wqb.bitcast(jnp.int32)
        wow = wob.bitcast(jnp.int32)
        w3w = w3b.bitcast(jnp.int32)
        w4w = w4b.bitcast(jnp.int32)

        SK, SV, SA = 0, 1, 2
        SX, SWQ, SWO, SW3, SW4 = SV, SA, SK, SV, SA

        def start_w(src, dst, sem):
            for n in range(dst.shape[0]):
                pltpu.make_async_copy(src.at[:, n * LANE:(n + 1) * LANE],
                                      dst.at[n], sems.at[sem]).start()

        def start_wo():
            rc = HD // WOC
            for r in range(WOC):
                for n in range(ND):
                    pltpu.make_async_copy(
                        wo_hbm.at[r * rc:(r + 1) * rc, n * LANE:(n + 1) * LANE],
                        wob.at[n, r * rc:(r + 1) * rc, :], sems.at[SWO]).start()

        def wait_all(dst, sem):
            pltpu.make_async_copy(dst, dst, sems.at[sem]).wait()

        def start_w4():
            for ch in range(W4C):
                for n in range(ND):
                    pltpu.make_async_copy(
                        w4_hbm.at[W4E[ch]:W4E[ch + 1], n * LANE:(n + 1) * LANE],
                        w4b.at[n, W4E[ch]:W4E[ch + 1], :],
                        sems.at[SW4 + ch]).start()

        def wait_w4(ch):
            wait_all(w4b.at[:, W4E[ch]:W4E[ch + 1], :], SW4 + ch)

        def start_kv(src, dst, g, sem):
            r0 = pl.multiple_of(g * GR, GR)
            for c in range(ns):
                pltpu.make_async_copy(
                    src.at[pl.ds(r0, GR), pl.ds(s0 + c * LANE, LANE)],
                    dst.at[c, pl.ds(r0, GR), :], sems.at[sem]).start()

        def wait_kv(dst, g, sem):
            r0 = pl.multiple_of(g * GR, GR)
            wait_all(dst.at[:, pl.ds(r0, GR), :], sem)

        pltpu.make_async_copy(x_hbm, xb, sems.at[SX]).start()
        start_w(wq_hbm, wqb, SWQ)
        start_kv(k_hbm, kb, 0, SK)
        wait_all(xb, SX)
        x0 = xb[...].astype(jnp.float32)

        row = jax.lax.broadcasted_iota(jnp.int32, (G, LANE), 0)
        lane = jax.lax.broadcasted_iota(jnp.int32, (G, LANE), 1)

        def head_mask(t):
            j, r = divmod(t, 3)
            if r == 0:
                return row == 2 * j
            if r == 2:
                return row == 2 * j + 1
            return row == jnp.where(lane >= 64, 2 * j + 1, 2 * j)

        masks = [head_mask(t) for t in range(NT)]

        def ln_stats(x):
            m = jnp.mean(x, axis=-1, keepdims=True)
            v = jnp.maximum(jnp.mean(x * x, axis=-1, keepdims=True) - m * m, 0.0)
            return x - m, v

        def mixer(x, streaming):
            xc, v = ln_stats(x)
            r1 = jax.lax.rsqrt(v + EPS)
            x1 = xc * r1
            hn = x1 * jax.lax.rsqrt(v * r1 * r1 + EPS)
            hn = jnp.broadcast_to(hn, (G, D)).astype(jnp.bfloat16)
            if streaming:
                wait_all(w3b, SW3)
            h = jnp.concatenate(
                [_gelu(_dot(hn, _bf(w3w[n]))) for n in range(F // LANE)],
                axis=1).astype(jnp.bfloat16)
            hs = [None] * ND
            for ch in range(W4C):
                if streaming:
                    wait_w4(ch)
                for n in range(ND):
                    hs[n] = _acc(hs[n], _dot(
                        h[:, W4E[ch]:W4E[ch + 1]],
                        _bf(w4w[n, W4E[ch] // 2:W4E[ch + 1] // 2, :])))
            return x + x1 + jnp.concatenate(hs, axis=1)[0:1, :]

        def q_store(g, t, q):
            qb[g, :, t * LANE:(t + 1) * LANE] = _words(jnp.where(masks[t], q, 0.0))

        def layer1(x):
            xc, v = ln_stats(x)
            xn8 = jnp.broadcast_to(xc * jax.lax.rsqrt(v + EPS),
                                   (G, D)).astype(jnp.bfloat16)
            wait_all(wqb, SWQ)
            start_kv(v_hbm, vb, 0, SV)
            for n in range(HD // LANE):
                q_store(n // NT, n % NT, _dot(xn8, _bf(wqw[n])) * scale)

            def trq(n, _):
                blk = _bf(wqw[n])
                wqw[n] = jnp.concatenate(
                    [pltpu.bitcast(blk[kt * LANE:(kt + 1) * LANE, :].T, jnp.int32)
                     for kt in range(ND)], axis=0)
                return 0

            jax.lax.fori_loop(MT, HD // LANE, trq, 0)

            def group(g, _):
                wait_kv(kb, g, SK)

                @pl.when(g + 1 < NG)
                def _():
                    start_kv(k_hbm, kb, g + 1, SK)

                @pl.when(g + 1 == NG)
                def _():
                    start_wo()

                rw = pl.multiple_of(g * (GR // 2), GR // 2)
                qg = _bf(qb[g])
                mx = None
                for c in range(ns):
                    s = _dot(qg, _bf(kw[c, pl.ds(rw, GR // 2), :]))[0:G]
                    sa[g, c] = s
                    mx = s if mx is None else jnp.maximum(mx, s)
                m = jnp.max(mx, axis=1, keepdims=True)

                wait_kv(vb, g, SV)

                @pl.when(g + 1 < NG)
                def _():
                    start_kv(v_hbm, vb, g + 1, SV)

                @pl.when(g + 1 == NG)
                def _():
                    start_w(w3_hbm, w3b, SW3)
                    start_w4()

                lsum = None
                acc = None
                for c in range(ns):
                    p = jnp.exp(sa[g, c] - m)
                    lsum = _acc(lsum, p)
                    acc = _acc(acc, _dot_nt(p.astype(jnp.bfloat16),
                                            _bf(vw[c, pl.ds(rw, GR // 2), :])))
                inv = 1.0 / _lanesum(lsum)
                for t in range(NT):
                    ob[g, :, t * LANE:(t + 1) * LANE] = _words(jnp.where(
                        masks[t], acc[:, t * LANE:(t + 1) * LANE] * inv, 0.0))

                def retile(t0, nt):
                    def tr(c, _):
                        r0 = pl.multiple_of(g * (GR // 2) + t0 * (LANE // 2), LANE // 2)
                        blk = _bf(vw[c, pl.ds(r0, nt * LANE // 2), :])
                        vw[c, pl.ds(r0, nt * LANE // 2), :] = jnp.concatenate(
                            [pltpu.bitcast(blk[t * LANE:(t + 1) * LANE, :].T, jnp.int32)
                             for t in range(nt)], axis=0)
                        return 0
                    jax.lax.fori_loop(0, ns, tr, 0)

                def blocks(i, _):
                    retile(i * TRB, TRB)
                    return 0

                nblk = jnp.clip(MT // TRB - g * (NT // TRB), 0, NT // TRB)
                jax.lax.fori_loop(0, nblk, blocks, 0)
                return 0

            jax.lax.fori_loop(0, NG, group, 0)
            wait_all(wob, SWO)
            ys = [None] * ND
            for g in range(NG):
                og = _bf(ob[g])
                for n in range(ND):
                    ys[n] = _acc(ys[n], _dot(
                        og, _bf(wow[n, g * (GR // 2):(g + 1) * (GR // 2), :]))[0:G])
            x = x + jnp.concatenate(
                [jnp.sum(y, axis=0, keepdims=True) for y in ys], axis=1)
            return mixer(x, True)

        def layer2(x):
            xc, v = ln_stats(x)
            xn = xc * jax.lax.rsqrt(v + EPS)
            xn8 = jnp.broadcast_to(xn, (G, D)).astype(jnp.bfloat16)

            xs = xn * scale
            xr = [jnp.broadcast_to(xs[:, kt * LANE:(kt + 1) * LANE], (G, LANE))
                  for kt in range(ND)]
            tasks_m, tasks_v = [], []
            for n in range(MT):
                def tm(n=n):
                    q_store(n // NT, n % NT, _dot(xn8, _bf(wqw[n])) * scale)
                tasks_m.append(tm)
            for n in range(MT, HD // LANE):
                for r in range(LANE // 16):
                    def tv(n=n, r=r):
                        a0 = a1 = None
                        for kt in range(ND):
                            w0, w1 = _f32(wqw[n, kt * 64 + r * 8:kt * 64 + r * 8 + 8, :])
                            a0 = _acc(a0, w0 * xr[kt])
                            a1 = _acc(a1, w1 * xr[kt])
                        r0 = (n - MT) * LANE + r * 16
                        qc[r0:r0 + 8, :] = jnp.broadcast_to(_lanesum(a0), (G, LANE))
                        qc[r0 + 8:r0 + 16, :] = jnp.broadcast_to(_lanesum(a1), (G, LANE))
                    tasks_v.append(tv)
            _interleave(tasks_m, tasks_v)
            acc_b[...] = jnp.zeros(acc_b.shape, jnp.float32)

            def qk_body(b, _):
                c0 = b * sb_n
                tasks_m, tasks_v = [], []
                for ci in range(sb_n):
                    for t0 in range(0, MT, NT):
                        def tm(ci=ci, t0=t0):
                            c = c0 + ci
                            g = t0 // NT
                            nt = min(NT, MT - t0)
                            q = _bf(qb[g])
                            kc = _bf(kw[c, t0 * 64:(t0 + nt) * 64, :])
                            for t in range(nt):
                                r = _dot(q[:, t * LANE:(t + 1) * LANE],
                                         kc[t * LANE:(t + 1) * LANE, :])
                                jj, kind = divmod(t, 3)
                                if kind == 0:
                                    sa[g, c, 2 * jj:2 * jj + 1, :] = r[2 * jj:2 * jj + 1, :]
                                elif kind == 2:
                                    sa[g, c, 2 * jj + 1:2 * jj + 2, :] = r[2 * jj + 1:2 * jj + 2, :]
                                else:
                                    sb[g, c, 2 * jj:2 * jj + 2, :] = r[2 * jj:2 * jj + 2, :]
                        tasks_m.append(tm)
                for hv in range(NV):
                    def tv(hv=hv):
                        h = NM + hv
                        qs = [qc[(hv * 24 + j) * 8:(hv * 24 + j + 1) * 8, :]
                              for j in range(24)]
                        for ci in range(sb_n):
                            c = c0 + ci
                            blk = kw[c, h * 96:(h + 1) * 96, :]
                            a0 = a1 = None
                            for d in range(12):
                                k0, k1 = _f32(blk[d * 8:(d + 1) * 8, :])
                                a0 = _acc(a0, k0 * qs[2 * d])
                                a1 = _acc(a1, k1 * qs[2 * d + 1])
                            sa[h // G, c, h % G:h % G + 1, :] = jnp.sum(
                                a0 + a1, axis=0, keepdims=True)
                    tasks_v.append(tv)
                _interleave(tasks_m, tasks_v)
                return 0

            jax.lax.fori_loop(0, ns // sb_n, qk_body, 0)

            invs = []
            for g in range(NG):
                n_m = min(max(NM - g * G, 0), G)
                ss = []
                mx = None
                for c in range(ns):
                    s = sa[g, c]
                    if n_m:
                        s = s + sb[g, c]
                    ss.append(s)
                    mx = s if mx is None else jnp.maximum(mx, s)
                m = jnp.max(mx, axis=1, keepdims=True)
                lsum = None
                for c in range(ns):
                    e = jnp.exp(ss[c] - m)
                    lsum = _acc(lsum, e)
                    if n_m:
                        pb[g, c] = _words(e)
                    if n_m < G:
                        sa[g, c] = e
                invs.append(1.0 / _lanesum(lsum))

            def pv_body(b, _):
                c0 = b * sb_n
                tasks_m, tasks_v = [], []
                for ci in range(sb_n):
                    for t0 in range(0, MT, NT):
                        def tm(ci=ci, t0=t0):
                            c = c0 + ci
                            g = t0 // NT
                            nt = min(NT, MT - t0)
                            p = _bf(pb[g, c])
                            vc = _bf(vw[c, t0 * 64:(t0 + nt) * 64, :])
                            for t in range(nt):
                                part[c, t0 + t] = _dot(
                                    p, vc[t * LANE:(t + 1) * LANE, :])[0:G]
                        tasks_m.append(tm)
                for hv in range(NV):
                    def tv(hv=hv):
                        h = NM + hv
                        ps = [jnp.broadcast_to(
                            sa[h // G, c0 + ci, h % G:h % G + 1, :], (G, LANE))
                            for ci in range(sb_n)]
                        for d in range(12):
                            a0 = a1 = None
                            for ci in range(sb_n):
                                v0, v1 = _f32(vw[c0 + ci,
                                                 h * 96 + d * 8:h * 96 + d * 8 + 8, :])
                                a0 = _acc(a0, v0 * ps[ci])
                                a1 = _acc(a1, v1 * ps[ci])
                            r = hv * DH + d * 16
                            acc_b[r:r + 8, :] = acc_b[r:r + 8, :] + a0
                            acc_b[r + 8:r + 16, :] = acc_b[r + 8:r + 16, :] + a1
                    tasks_v.append(tv)
                _interleave(tasks_m, tasks_v)
                return 0

            jax.lax.fori_loop(0, ns // sb_n, pv_body, 0)

            for n in range(MT):
                g, t = divmod(n, NT)
                tot = None
                for c in range(ns):
                    tot = _acc(tot, part[c, n])
                ob[g, :, t * LANE:(t + 1) * LANE] = _words(
                    jnp.where(masks[t], tot * invs[g], 0.0))

            ys = [None] * ND
            yv = [None] * ND
            tasks_m, tasks_v = [], []
            for kt in range(MT):
                def tm(kt=kt):
                    g, t = divmod(kt, NT)
                    og = _bf(ob[g, :, t * LANE:(t + 1) * LANE])
                    for n in range(ND):
                        ys[n] = _acc(ys[n], _dot(
                            og, _bf(wow[n, kt * 64:(kt + 1) * 64, :]))[0:G])
                tasks_m.append(tm)
            for hv in range(NV):
                def tv(hv=hv):
                    h = NM + hv
                    inv = jnp.broadcast_to(invs[h // G][h % G:h % G + 1, :], (G, LANE))
                    for d in range(12):
                        r = hv * DH + d * 16
                        o0 = _lanesum(acc_b[r:r + 8, :]) * inv
                        o1 = _lanesum(acc_b[r + 8:r + 16, :]) * inv
                        for n in range(ND):
                            w0, w1 = _f32(wow[n, h * 96 + d * 8:h * 96 + d * 8 + 8, :])
                            yv[n] = _acc(yv[n], w0 * o0 + w1 * o1)
                tasks_v.append(tv)
            _interleave(tasks_m, tasks_v)
            x = x + jnp.concatenate(
                [jnp.sum(a + b, axis=0, keepdims=True) for a, b in zip(ys, yv)],
                axis=1)
            return mixer(x, False)

        sb[...] = jnp.zeros(sb.shape, jnp.float32)
        o_ref[...] = layer2(layer1(x0)).astype(o_ref.dtype)

    return kernel


@jax.jit
def pallas_interleave_layers__sliding_block_cached__mixer_s_mlp__decode_kernel(
    A_x: jax.Array,
    A_k_cache: jax.Array,
    A_v_cache: jax.Array,
    A_wq: jax.Array,
    A_wo: jax.Array,
    B_x: jax.Array,
    B_w1: jax.Array,
    B_w2: jax.Array,
    B_w3: jax.Array,
    B_w4: jax.Array,
):
    del B_x, B_w1, B_w2
    sk = A_k_cache.shape[2]
    w = min(4096, max(256, sk // 4))
    ns = w // LANE
    k_t = jnp.transpose(A_k_cache, (0, 1, 3, 2)).reshape(HD, sk)
    v_t = jnp.transpose(A_v_cache, (0, 1, 3, 2)).reshape(HD, sk)
    x2 = A_x.reshape(1, D)

    any_spec = pl.BlockSpec(memory_space=pl.ANY)
    out = pl.pallas_call(
        _make_kernel(sk, w),
        in_specs=[any_spec] * 7,
        out_specs=pl.BlockSpec(memory_space=pltpu.VMEM),
        out_shape=jax.ShapeDtypeStruct((1, D), A_x.dtype),
        scratch_shapes=[
            pltpu.VMEM((1, D), jnp.bfloat16),
            pltpu.VMEM((ns, HD, LANE), jnp.bfloat16),
            pltpu.VMEM((ns, HD, LANE), jnp.bfloat16),
            pltpu.VMEM((HD // LANE, D, LANE), jnp.bfloat16),
            pltpu.VMEM((ND, HD, LANE), jnp.bfloat16),
            pltpu.VMEM((F // LANE, D, LANE), jnp.bfloat16),
            pltpu.VMEM((ND, F, LANE), jnp.bfloat16),
            pltpu.VMEM((NG, G, GR), jnp.int32),
            pltpu.VMEM((NG, ns, G, LANE), jnp.float32),
            pltpu.VMEM((NG, ns, G, LANE), jnp.float32),
            pltpu.VMEM((NG, ns, G, LANE), jnp.int32),
            pltpu.VMEM((NV * DH, LANE), jnp.float32),
            pltpu.VMEM((NV * DH, LANE), jnp.float32),
            pltpu.VMEM((ns, MT, G, LANE), jnp.float32),
            pltpu.VMEM((NG, G, GR), jnp.int32),
            pltpu.SemaphoreType.DMA((2 + W4C,)),
        ],
        compiler_params=pltpu.CompilerParams(
            vmem_limit_bytes=128 * 1024 * 1024),
    )(x2, k_t, v_t, A_wq, A_wo, B_w3, B_w4)
    return out.reshape(A_x.shape)
```

```python
import jax
import jax.numpy as jnp
import jax.experimental.pallas as pl
import jax.experimental.pallas.tpu as pltpu

H, DH, D, F = 32, 192, 640, 1536
HD = H * DH
G = 8
NG = H // G
GR = G * DH
LANE = 128
NT = GR // LANE
ND = D // LANE
EPS = 1e-5

NV = 12
NM = H - NV
MT = NM * DH // LANE
MG = -(-MT // NT)
SB = 16
TRB = 3
W4E = (0, 640, 1280, 1536)
W4C = len(W4E) - 1
WOC = 8


def _gelu(x):
    c = 0.7978845608028654
    return 0.5 * x * (1.0 + jnp.tanh(c * (x + 0.044715 * (x * x * x))))


def _bf(w):
    return pltpu.bitcast(w, jnp.bfloat16)


def _f32(w):
    x = _bf(w).astype(jnp.float32)
    return x[0:8], x[8:16]


def _words(x8):
    x16 = jnp.concatenate([x8, jnp.zeros_like(x8)], axis=0).astype(jnp.bfloat16)
    return pltpu.bitcast(x16, jnp.int32)


def _dot(a, b):
    return jnp.dot(a, b, preferred_element_type=jnp.float32)


def _dot_nt(a, b):
    return jax.lax.dot_general(a, b, (((1,), (1,)), ((), ())),
                               preferred_element_type=jnp.float32)


def _acc(a, b):
    return b if a is None else a + b


def _lanesum(a):
    return jnp.sum(a, axis=1, keepdims=True)


def _row_store(ref, g, c, t, r):
    j, kind = divmod(t, 3)
    if kind == 0:
        ref[0, g, c, 2 * j:2 * j + 1, :] = r[2 * j:2 * j + 1, :]
    elif kind == 2:
        ref[0, g, c, 2 * j + 1:2 * j + 2, :] = r[2 * j + 1:2 * j + 2, :]
    else:
        ref[1, g, c, 2 * j:2 * j + 2, :] = r[2 * j:2 * j + 2, :]


def _interleave(tasks_m, tasks_v):
    nm, nv = len(tasks_m), len(tasks_v)
    im = 0
    for iv in range(nv):
        while im < nm and im * nv <= iv * nm:
            tasks_m[im]()
            im += 1
        tasks_v[iv]()
    while im < nm:
        tasks_m[im]()
        im += 1


def _make_kernel(sk, w):
    ns = w // LANE
    s0 = sk - w
    sb_n = min(SB, ns)
    scale = DH ** -0.5

    def kernel(x_hbm, k_hbm, v_hbm, wq_hbm, wo_hbm, w3_hbm, w4_hbm, o_ref,
               xb, kb, vb, wqb, wob, w3b, w4b, qb, sc, pb, qc, acc_b, part,
               ob, sems):
        kw = kb.bitcast(jnp.int32)
        vw = vb.bitcast(jnp.int32)
        wqw = wqb.bitcast(jnp.int32)
        wow = wob.bitcast(jnp.int32)
        w3w = w3b.bitcast(jnp.int32)
        w4w = w4b.bitcast(jnp.int32)

        SK, SV, SA = 0, 1, 2
        SX, SWQ, SWO, SW3, SW4 = SV, SA, SK, SV, SA

        def start_w(src, dst, sem):
            for n in range(dst.shape[0]):
                pltpu.make_async_copy(src.at[:, n * LANE:(n + 1) * LANE],
                                      dst.at[n], sems.at[sem]).start()

        def start_wo():
            rc = HD // WOC
            for r in range(WOC):
                for n in range(ND):
                    pltpu.make_async_copy(
                        wo_hbm.at[r * rc:(r + 1) * rc, n * LANE:(n + 1) * LANE],
                        wob.at[n, r * rc:(r + 1) * rc, :], sems.at[SWO]).start()

        def wait_all(dst, sem):
            pltpu.make_async_copy(dst, dst, sems.at[sem]).wait()

        def start_w4():
            for ch in range(W4C):
                for n in range(ND):
                    pltpu.make_async_copy(
                        w4_hbm.at[W4E[ch]:W4E[ch + 1], n * LANE:(n + 1) * LANE],
                        w4b.at[n, W4E[ch]:W4E[ch + 1], :],
                        sems.at[SW4 + ch]).start()

        def wait_w4(ch):
            wait_all(w4b.at[:, W4E[ch]:W4E[ch + 1], :], SW4 + ch)

        def start_kv(src, dst, g, sem):
            r0 = pl.multiple_of(g * GR, GR)
            for c in range(ns):
                pltpu.make_async_copy(
                    src.at[pl.ds(r0, GR), pl.ds(s0 + c * LANE, LANE)],
                    dst.at[c, pl.ds(r0, GR), :], sems.at[sem]).start()

        def wait_kv(dst, g, sem):
            r0 = pl.multiple_of(g * GR, GR)
            wait_all(dst.at[:, pl.ds(r0, GR), :], sem)

        pltpu.make_async_copy(x_hbm, xb, sems.at[SX]).start()
        start_w(wq_hbm, wqb, SWQ)
        start_kv(k_hbm, kb, 0, SK)
        wait_all(xb, SX)
        x0 = xb[...].astype(jnp.float32)

        row = jax.lax.broadcasted_iota(jnp.int32, (G, LANE), 0)
        lane = jax.lax.broadcasted_iota(jnp.int32, (G, LANE), 1)

        def head_mask(t):
            j, r = divmod(t, 3)
            if r == 0:
                return row == 2 * j
            if r == 2:
                return row == 2 * j + 1
            return row == jnp.where(lane >= 64, 2 * j + 1, 2 * j)

        masks = [head_mask(t) for t in range(NT)]

        def ln_stats(x):
            m = jnp.mean(x, axis=-1, keepdims=True)
            v = jnp.maximum(jnp.mean(x * x, axis=-1, keepdims=True) - m * m, 0.0)
            return x - m, v

        def mixer(x, streaming):
            xc, v = ln_stats(x)
            r1 = jax.lax.rsqrt(v + EPS)
            x1 = xc * r1
            hn = x1 * jax.lax.rsqrt(v * r1 * r1 + EPS)
            hn = jnp.broadcast_to(hn, (G, D)).astype(jnp.bfloat16)
            if streaming:
                wait_all(w3b, SW3)
            h = jnp.concatenate(
                [_gelu(_dot(hn, _bf(w3w[n]))) for n in range(F // LANE)],
                axis=1).astype(jnp.bfloat16)
            hs = [None] * ND
            for ch in range(W4C):
                if streaming:
                    wait_w4(ch)
                for n in range(ND):
                    hs[n] = _acc(hs[n], _dot(
                        h[:, W4E[ch]:W4E[ch + 1]],
                        _bf(w4w[n, W4E[ch] // 2:W4E[ch + 1] // 2, :])))
            return x + x1 + jnp.concatenate(hs, axis=1)[0:1, :]

        def q_store(g, t, q):
            qb[g, :, t * LANE:(t + 1) * LANE] = _words(jnp.where(masks[t], q, 0.0))

        def layer1(x):
            xc, v = ln_stats(x)
            xn8 = jnp.broadcast_to(xc * jax.lax.rsqrt(v + EPS),
                                   (G, D)).astype(jnp.bfloat16)
            wait_all(wqb, SWQ)
            start_kv(v_hbm, vb, 0, SV)
            for n in range(HD // LANE):
                q_store(n // NT, n % NT, _dot(xn8, _bf(wqw[n])) * scale)

            def trq(n, _):
                blk = _bf(wqw[n])
                wqw[n] = jnp.concatenate(
                    [pltpu.bitcast(blk[kt * LANE:(kt + 1) * LANE, :].T, jnp.int32)
                     for kt in range(ND)], axis=0)
                return 0

            jax.lax.fori_loop(MT, HD // LANE, trq, 0)

            def group(g, _):
                wait_kv(kb, g, SK)

                @pl.when(g + 1 < NG)
                def _():
                    start_kv(k_hbm, kb, g + 1, SK)

                @pl.when(g + 1 == NG)
                def _():
                    start_wo()

                rw = pl.multiple_of(g * (GR // 2), GR // 2)
                qg = _bf(qb[g])
                mx = None
                for c in range(ns):
                    s = _dot(qg, _bf(kw[c, pl.ds(rw, GR // 2), :]))[0:G]
                    sc[0, g, c] = s
                    mx = s if mx is None else jnp.maximum(mx, s)
                m = jnp.max(mx, axis=1, keepdims=True)

                wait_kv(vb, g, SV)

                @pl.when(g + 1 < NG)
                def _():
                    start_kv(v_hbm, vb, g + 1, SV)

                @pl.when(g + 1 == NG)
                def _():
                    start_w(w3_hbm, w3b, SW3)
                    start_w4()

                lsum = None
                acc = None
                for c in range(ns):
                    p = jnp.exp(sc[0, g, c] - m)
                    lsum = _acc(lsum, p)
                    acc = _acc(acc, _dot_nt(p.astype(jnp.bfloat16),
                                            _bf(vw[c, pl.ds(rw, GR // 2), :])))
                inv = 1.0 / _lanesum(lsum)
                for t in range(NT):
                    ob[g, :, t * LANE:(t + 1) * LANE] = _words(jnp.where(
                        masks[t], acc[:, t * LANE:(t + 1) * LANE] * inv, 0.0))

                def retile(t0, nt):
                    def tr(c, _):
                        r0 = pl.multiple_of(g * (GR // 2) + t0 * (LANE // 2), LANE // 2)
                        blk = _bf(vw[c, pl.ds(r0, nt * LANE // 2), :])
                        vw[c, pl.ds(r0, nt * LANE // 2), :] = jnp.concatenate(
                            [pltpu.bitcast(blk[t * LANE:(t + 1) * LANE, :].T, jnp.int32)
                             for t in range(nt)], axis=0)
                        return 0
                    jax.lax.fori_loop(0, ns, tr, 0)

                def blocks(i, _):
                    retile(i * TRB, TRB)
                    return 0

                nblk = jnp.clip(MT // TRB - g * (NT // TRB), 0, NT // TRB)
                jax.lax.fori_loop(0, nblk, blocks, 0)
                return 0

            jax.lax.fori_loop(0, NG, group, 0)
            wait_all(wob, SWO)
            ys = [None] * ND
            for g in range(NG):
                og = _bf(ob[g])
                for n in range(ND):
                    ys[n] = _acc(ys[n], _dot(
                        og, _bf(wow[n, g * (GR // 2):(g + 1) * (GR // 2), :]))[0:G])
            x = x + jnp.concatenate(
                [jnp.sum(y, axis=0, keepdims=True) for y in ys], axis=1)
            return mixer(x, True)

        def layer2(x):
            xc, v = ln_stats(x)
            xn = xc * jax.lax.rsqrt(v + EPS)
            xn8 = jnp.broadcast_to(xn, (G, D)).astype(jnp.bfloat16)

            xs = xn * scale
            xr = [jnp.broadcast_to(xs[:, kt * LANE:(kt + 1) * LANE], (G, LANE))
                  for kt in range(ND)]
            tasks_m, tasks_v = [], []
            for n in range(MT):
                def tm(n=n):
                    q_store(n // NT, n % NT, _dot(xn8, _bf(wqw[n])) * scale)
                tasks_m.append(tm)
            for n in range(MT, HD // LANE):
                for r in range(LANE // 16):
                    def tv(n=n, r=r):
                        a0 = a1 = None
                        for kt in range(ND):
                            w0, w1 = _f32(wqw[n, kt * 64 + r * 8:kt * 64 + r * 8 + 8, :])
                            a0 = _acc(a0, w0 * xr[kt])
                            a1 = _acc(a1, w1 * xr[kt])
                        r0 = (n - MT) * LANE + r * 16
                        qc[r0:r0 + 8, :] = jnp.broadcast_to(_lanesum(a0), (G, LANE))
                        qc[r0 + 8:r0 + 16, :] = jnp.broadcast_to(_lanesum(a1), (G, LANE))
                    tasks_v.append(tv)
            _interleave(tasks_m, tasks_v)
            acc_b[...] = jnp.zeros(acc_b.shape, jnp.float32)

            def qk_body(b, _):
                c0 = b * sb_n
                tasks_m, tasks_v = [], []
                for ci in range(sb_n):
                    for t0 in range(0, MT, NT):
                        def tm(ci=ci, t0=t0):
                            c = c0 + ci
                            g = t0 // NT
                            nt = min(NT, MT - t0)
                            q = _bf(qb[g])
                            kc = _bf(kw[c, t0 * 64:(t0 + nt) * 64, :])
                            for t in range(nt):
                                _row_store(sc, g, c, t, _dot(
                                    q[:, t * LANE:(t + 1) * LANE],
                                    kc[t * LANE:(t + 1) * LANE, :]))
                        tasks_m.append(tm)
                for hv in range(NV):
                    def tv(hv=hv):
                        h = NM + hv
                        qs = [qc[(hv * 24 + j) * 8:(hv * 24 + j + 1) * 8, :]
                              for j in range(24)]
                        for ci in range(sb_n):
                            c = c0 + ci
                            blk = kw[c, h * 96:(h + 1) * 96, :]
                            a0 = a1 = None
                            for d in range(12):
                                k0, k1 = _f32(blk[d * 8:(d + 1) * 8, :])
                                a0 = _acc(a0, k0 * qs[2 * d])
                                a1 = _acc(a1, k1 * qs[2 * d + 1])
                            sc[0, h // G, c, h % G:h % G + 1, :] = jnp.sum(
                                a0 + a1, axis=0, keepdims=True)
                    tasks_v.append(tv)
                _interleave(tasks_m, tasks_v)
                return 0

            jax.lax.fori_loop(0, ns // sb_n, qk_body, 0)

            invs = []
            for g in range(NG):
                n_m = min(max(NM - g * G, 0), G)
                ss = []
                mx = None
                for c in range(ns):
                    s = sc[0, g, c]
                    if n_m:
                        s = s + sc[1, g, c]
                    ss.append(s)
                    mx = s if mx is None else jnp.maximum(mx, s)
                m = jnp.max(mx, axis=1, keepdims=True)
                lsum = None
                for c in range(ns):
                    e = jnp.exp(ss[c] - m)
                    lsum = _acc(lsum, e)
                    if n_m:
                        pb[g, c] = _words(e)
                    if n_m < G:
                        sc[0, g, c] = e
                invs.append(1.0 / _lanesum(lsum))

            def pv_body(b, _):
                c0 = b * sb_n
                tasks_m, tasks_v = [], []
                for ci in range(sb_n):
                    for t0 in range(0, MT, NT):
                        def tm(ci=ci, t0=t0):
                            c = c0 + ci
                            g = t0 // NT
                            nt = min(NT, MT - t0)
                            p = _bf(pb[g, c])
                            vc = _bf(vw[c, t0 * 64:(t0 + nt) * 64, :])
                            for t in range(nt):
                                _row_store(part, g, c, t,
                                           _dot(p, vc[t * LANE:(t + 1) * LANE, :]))
                        tasks_m.append(tm)
                for hv in range(NV):
                    def tv(hv=hv):
                        h = NM + hv
                        ps = [jnp.broadcast_to(
                            sc[0, h // G, c0 + ci, h % G:h % G + 1, :], (G, LANE))
                            for ci in range(sb_n)]
                        for d in range(12):
                            a0 = a1 = None
                            for ci in range(sb_n):
                                v0, v1 = _f32(vw[c0 + ci,
                                                 h * 96 + d * 8:h * 96 + d * 8 + 8, :])
                                a0 = _acc(a0, v0 * ps[ci])
                                a1 = _acc(a1, v1 * ps[ci])
                            r = hv * DH + d * 16
                            acc_b[r:r + 8, :] = acc_b[r:r + 8, :] + a0
                            acc_b[r + 8:r + 16, :] = acc_b[r + 8:r + 16, :] + a1
                    tasks_v.append(tv)
                _interleave(tasks_m, tasks_v)
                return 0

            jax.lax.fori_loop(0, ns // sb_n, pv_body, 0)

            for g in range(MG):
                tot = [None, None]
                for c in range(ns):
                    tot = [_acc(tot[i], part[i, g, c]) for i in range(2)]
                tot = [a * invs[g] for a in tot]
                for t in range(min(NT, MT - g * NT)):
                    ob[g, :, t * LANE:(t + 1) * LANE] = _words(
                        jnp.where(masks[t], tot[1 if t % 3 == 1 else 0], 0.0))

            ys = [None] * ND
            yv = [None] * ND
            tasks_m, tasks_v = [], []
            for kt in range(MT):
                def tm(kt=kt):
                    g, t = divmod(kt, NT)
                    og = _bf(ob[g, :, t * LANE:(t + 1) * LANE])
                    for n in range(ND):
                        ys[n] = _acc(ys[n], _dot(
                            og, _bf(wow[n, kt * 64:(kt + 1) * 64, :]))[0:G])
                tasks_m.append(tm)
            for hv in range(NV):
                def tv(hv=hv):
                    h = NM + hv
                    inv = jnp.broadcast_to(invs[h // G][h % G:h % G + 1, :], (G, LANE))
                    for d in range(12):
                        r = hv * DH + d * 16
                        o0 = _lanesum(acc_b[r:r + 8, :]) * inv
                        o1 = _lanesum(acc_b[r + 8:r + 16, :]) * inv
                        for n in range(ND):
                            w0, w1 = _f32(wow[n, h * 96 + d * 8:h * 96 + d * 8 + 8, :])
                            yv[n] = _acc(yv[n], w0 * o0 + w1 * o1)
                tasks_v.append(tv)
            _interleave(tasks_m, tasks_v)
            x = x + jnp.concatenate(
                [jnp.sum(a + b, axis=0, keepdims=True) for a, b in zip(ys, yv)],
                axis=1)
            return mixer(x, False)

        sc[1] = jnp.zeros(sc.shape[1:], jnp.float32)
        part[...] = jnp.zeros(part.shape, jnp.float32)
        o_ref[...] = layer2(layer1(x0)).astype(o_ref.dtype)

    return kernel


@jax.jit
def pallas_interleave_layers__sliding_block_cached__mixer_s_mlp__decode_kernel(
    A_x: jax.Array,
    A_k_cache: jax.Array,
    A_v_cache: jax.Array,
    A_wq: jax.Array,
    A_wo: jax.Array,
    B_x: jax.Array,
    B_w1: jax.Array,
    B_w2: jax.Array,
    B_w3: jax.Array,
    B_w4: jax.Array,
):
    del B_x, B_w1, B_w2
    sk = A_k_cache.shape[2]
    w = min(4096, max(256, sk // 4))
    ns = w // LANE
    k_t = jnp.transpose(A_k_cache, (0, 1, 3, 2)).reshape(HD, sk)
    v_t = jnp.transpose(A_v_cache, (0, 1, 3, 2)).reshape(HD, sk)
    x2 = A_x.reshape(1, D)

    any_spec = pl.BlockSpec(memory_space=pl.ANY)
    out = pl.pallas_call(
        _make_kernel(sk, w),
        in_specs=[any_spec] * 7,
        out_specs=pl.BlockSpec(memory_space=pltpu.VMEM),
        out_shape=jax.ShapeDtypeStruct((1, D), A_x.dtype),
        scratch_shapes=[
            pltpu.VMEM((1, D), jnp.bfloat16),
            pltpu.VMEM((ns, HD, LANE), jnp.bfloat16),
            pltpu.VMEM((ns, HD, LANE), jnp.bfloat16),
            pltpu.VMEM((HD // LANE, D, LANE), jnp.bfloat16),
            pltpu.VMEM((ND, HD, LANE), jnp.bfloat16),
            pltpu.VMEM((F // LANE, D, LANE), jnp.bfloat16),
            pltpu.VMEM((ND, F, LANE), jnp.bfloat16),
            pltpu.VMEM((NG, G, GR), jnp.int32),
            pltpu.VMEM((2, NG, ns, G, LANE), jnp.float32),
            pltpu.VMEM((NG, ns, G, LANE), jnp.int32),
            pltpu.VMEM((NV * DH, LANE), jnp.float32),
            pltpu.VMEM((NV * DH, LANE), jnp.float32),
            pltpu.VMEM((2, MG, ns, G, LANE), jnp.float32),
            pltpu.VMEM((NG, G, GR), jnp.int32),
            pltpu.SemaphoreType.DMA((2 + W4C,)),
        ],
        compiler_params=pltpu.CompilerParams(
            vmem_limit_bytes=128 * 1024 * 1024),
    )(x2, k_t, v_t, A_wq, A_wo, B_w3, B_w4)
    return out.reshape(A_x.shape)
```

```python
import jax
import jax.numpy as jnp
import jax.experimental.pallas as pl
import jax.experimental.pallas.tpu as pltpu

H, DH, D, F = 32, 192, 640, 1536
HD = H * DH
G = 8
NG = H // G
GR = G * DH
LANE = 128
NT = GR // LANE
ND = D // LANE
EPS = 1e-5

NV = 12
NM = H - NV
MT = NM * DH // LANE
MG = -(-MT // NT)
SB = 16
TRB = 3
W4E = (0, 640, 1280, 1536)
W4C = len(W4E) - 1
WOC = 8


def _gelu(x):
    c = 0.7978845608028654
    return 0.5 * x * (1.0 + jnp.tanh(c * (x + 0.044715 * (x * x * x))))


def _bf(w):
    return pltpu.bitcast(w, jnp.bfloat16)


def _f32(w):
    x = _bf(w).astype(jnp.float32)
    return x[0:8], x[8:16]


def _words(x8):
    x16 = jnp.concatenate([x8, jnp.zeros_like(x8)], axis=0).astype(jnp.bfloat16)
    return pltpu.bitcast(x16, jnp.int32)


def _dot(a, b):
    return jnp.dot(a, b, preferred_element_type=jnp.float32)


def _dot_nt(a, b):
    return jax.lax.dot_general(a, b, (((1,), (1,)), ((), ())),
                               preferred_element_type=jnp.float32)


def _acc(a, b):
    return b if a is None else a + b


def _lanesum(a):
    return jnp.sum(a, axis=1, keepdims=True)


def _row_store(ref, g, c, t, r):
    j, kind = divmod(t, 3)
    if kind == 0:
        ref[0, g, c, 2 * j:2 * j + 1, :] = r[2 * j:2 * j + 1, :]
    elif kind == 2:
        ref[0, g, c, 2 * j + 1:2 * j + 2, :] = r[2 * j + 1:2 * j + 2, :]
    else:
        ref[1, g, c, 2 * j:2 * j + 2, :] = r[2 * j:2 * j + 2, :]


def _interleave(tasks_m, tasks_v):
    nm, nv = len(tasks_m), len(tasks_v)
    im = 0
    for iv in range(nv):
        while im < nm and im * nv <= iv * nm:
            tasks_m[im]()
            im += 1
        tasks_v[iv]()
    while im < nm:
        tasks_m[im]()
        im += 1


def _make_kernel(sk, w):
    ns = w // LANE
    s0 = sk - w
    sb_n = min(SB, ns)
    scale = DH ** -0.5

    def kernel(x_hbm, k_hbm, v_hbm, wq_hbm, wo_hbm, w3_hbm, w4_hbm, o_ref,
               xb, kb, vb, wqb, wob, w3b, w4b, qb, sc, pb, qc, acc_b, part,
               ob, sems):
        kw = kb.bitcast(jnp.int32)
        vw = vb.bitcast(jnp.int32)
        wqw = wqb.bitcast(jnp.int32)
        wow = wob.bitcast(jnp.int32)
        w3w = w3b.bitcast(jnp.int32)
        w4w = w4b.bitcast(jnp.int32)

        SK, SV, SA = 0, 1, 2
        SX, SWQ, SWO, SW3, SW4 = SV, SA, SK, SV, SA

        def start_w(src, dst, sem):
            for n in range(dst.shape[0]):
                pltpu.make_async_copy(src.at[:, n * LANE:(n + 1) * LANE],
                                      dst.at[n], sems.at[sem]).start()

        def start_wo():
            rc = HD // WOC
            for r in range(WOC):
                for n in range(ND):
                    pltpu.make_async_copy(
                        wo_hbm.at[r * rc:(r + 1) * rc, n * LANE:(n + 1) * LANE],
                        wob.at[n, r * rc:(r + 1) * rc, :], sems.at[SWO]).start()

        def wait_all(dst, sem):
            pltpu.make_async_copy(dst, dst, sems.at[sem]).wait()

        def start_w4():
            for ch in range(W4C):
                for n in range(ND):
                    pltpu.make_async_copy(
                        w4_hbm.at[W4E[ch]:W4E[ch + 1], n * LANE:(n + 1) * LANE],
                        w4b.at[n, W4E[ch]:W4E[ch + 1], :],
                        sems.at[SW4 + ch]).start()

        def wait_w4(ch):
            wait_all(w4b.at[:, W4E[ch]:W4E[ch + 1], :], SW4 + ch)

        def start_kv(src, dst, g, sem):
            r0 = pl.multiple_of(g * GR, GR)
            for c in range(ns):
                pltpu.make_async_copy(
                    src.at[pl.ds(r0, GR), pl.ds(s0 + c * LANE, LANE)],
                    dst.at[c, pl.ds(r0, GR), :], sems.at[sem]).start()

        def wait_kv(dst, g, sem):
            r0 = pl.multiple_of(g * GR, GR)
            wait_all(dst.at[:, pl.ds(r0, GR), :], sem)

        pltpu.make_async_copy(x_hbm, xb, sems.at[SX]).start()
        start_w(wq_hbm, wqb, SWQ)
        start_kv(k_hbm, kb, 0, SK)
        wait_all(xb, SX)
        x0 = xb[...].astype(jnp.float32)

        row = jax.lax.broadcasted_iota(jnp.int32, (G, LANE), 0)
        lane = jax.lax.broadcasted_iota(jnp.int32, (G, LANE), 1)

        def head_mask(t):
            j, r = divmod(t, 3)
            if r == 0:
                return row == 2 * j
            if r == 2:
                return row == 2 * j + 1
            return row == jnp.where(lane >= 64, 2 * j + 1, 2 * j)

        masks = [head_mask(t) for t in range(NT)]

        def ln_stats(x):
            xc = x - jnp.mean(x, axis=-1, keepdims=True)
            return xc, jnp.mean(xc * xc, axis=-1, keepdims=True)

        def mixer(x, streaming):
            xc, v = ln_stats(x)
            x1 = xc * jax.lax.rsqrt(v + EPS)
            xc, v = ln_stats(x1)
            hn = xc * jax.lax.rsqrt(v + EPS)
            hn = jnp.broadcast_to(hn, (G, D)).astype(jnp.bfloat16)
            if streaming:
                wait_all(w3b, SW3)
            h = jnp.concatenate(
                [_gelu(_dot(hn, _bf(w3w[n]))) for n in range(F // LANE)],
                axis=1).astype(jnp.bfloat16)
            hs = [None] * ND
            for ch in range(W4C):
                if streaming:
                    wait_w4(ch)
                for n in range(ND):
                    hs[n] = _acc(hs[n], _dot(
                        h[:, W4E[ch]:W4E[ch + 1]],
                        _bf(w4w[n, W4E[ch] // 2:W4E[ch + 1] // 2, :])))
            return x + x1 + jnp.concatenate(hs, axis=1)[0:1, :]

        def q_store(g, t, q):
            qb[g, :, t * LANE:(t + 1) * LANE] = _words(jnp.where(masks[t], q, 0.0))

        def layer1(x):
            xc, v = ln_stats(x)
            xn8 = jnp.broadcast_to(xc * jax.lax.rsqrt(v + EPS),
                                   (G, D)).astype(jnp.bfloat16)
            wait_all(wqb, SWQ)
            start_kv(v_hbm, vb, 0, SV)
            for n in range(HD // LANE):
                q_store(n // NT, n % NT, _dot(xn8, _bf(wqw[n])) * scale)

            def trq(n, _):
                blk = _bf(wqw[n])
                wqw[n] = jnp.concatenate(
                    [pltpu.bitcast(blk[kt * LANE:(kt + 1) * LANE, :].T, jnp.int32)
                     for kt in range(ND)], axis=0)
                return 0

            jax.lax.fori_loop(MT, HD // LANE, trq, 0)

            def group(g, _):
                wait_kv(kb, g, SK)

                @pl.when(g + 1 < NG)
                def _():
                    start_kv(k_hbm, kb, g + 1, SK)

                @pl.when(g + 1 == NG)
                def _():
                    start_wo()

                rw = pl.multiple_of(g * (GR // 2), GR // 2)
                qg = _bf(qb[g])
                mx = None
                for c in range(ns):
                    s = _dot(qg, _bf(kw[c, pl.ds(rw, GR // 2), :]))[0:G]
                    sc[0, g, c] = s
                    mx = s if mx is None else jnp.maximum(mx, s)
                m = jnp.max(mx, axis=1, keepdims=True)

                wait_kv(vb, g, SV)

                @pl.when(g + 1 < NG)
                def _():
                    start_kv(v_hbm, vb, g + 1, SV)

                @pl.when(g + 1 == NG)
                def _():
                    start_w(w3_hbm, w3b, SW3)
                    start_w4()

                lsum = None
                acc = None
                for c in range(ns):
                    p = jnp.exp(sc[0, g, c] - m)
                    lsum = _acc(lsum, p)
                    acc = _acc(acc, _dot_nt(p.astype(jnp.bfloat16),
                                            _bf(vw[c, pl.ds(rw, GR // 2), :])))
                inv = 1.0 / _lanesum(lsum)
                for t in range(NT):
                    ob[g, :, t * LANE:(t + 1) * LANE] = _words(jnp.where(
                        masks[t], acc[:, t * LANE:(t + 1) * LANE] * inv, 0.0))

                def retile(t0, nt):
                    def tr(c, _):
                        r0 = pl.multiple_of(g * (GR // 2) + t0 * (LANE // 2), LANE // 2)
                        blk = _bf(vw[c, pl.ds(r0, nt * LANE // 2), :])
                        vw[c, pl.ds(r0, nt * LANE // 2), :] = jnp.concatenate(
                            [pltpu.bitcast(blk[t * LANE:(t + 1) * LANE, :].T, jnp.int32)
                             for t in range(nt)], axis=0)
                        return 0
                    jax.lax.fori_loop(0, ns, tr, 0)

                def blocks(i, _):
                    retile(i * TRB, TRB)
                    return 0

                nblk = jnp.clip(MT // TRB - g * (NT // TRB), 0, NT // TRB)
                jax.lax.fori_loop(0, nblk, blocks, 0)
                return 0

            jax.lax.fori_loop(0, NG, group, 0)
            wait_all(wob, SWO)
            ys = [None] * ND
            for g in range(NG):
                og = _bf(ob[g])
                for n in range(ND):
                    ys[n] = _acc(ys[n], _dot(
                        og, _bf(wow[n, g * (GR // 2):(g + 1) * (GR // 2), :]))[0:G])
            x = x + jnp.concatenate(
                [jnp.sum(y, axis=0, keepdims=True) for y in ys], axis=1)
            return mixer(x, True)

        def layer2(x):
            xc, v = ln_stats(x)
            xn = xc * jax.lax.rsqrt(v + EPS)
            xn8 = jnp.broadcast_to(xn, (G, D)).astype(jnp.bfloat16)

            xs = xn * scale
            xr = [jnp.broadcast_to(xs[:, kt * LANE:(kt + 1) * LANE], (G, LANE))
                  for kt in range(ND)]
            tasks_m, tasks_v = [], []
            for n in range(MT):
                def tm(n=n):
                    q_store(n // NT, n % NT, _dot(xn8, _bf(wqw[n])) * scale)
                tasks_m.append(tm)
            for n in range(MT, HD // LANE):
                for r in range(LANE // 16):
                    def tv(n=n, r=r):
                        a0 = a1 = None
                        for kt in range(ND):
                            w0, w1 = _f32(wqw[n, kt * 64 + r * 8:kt * 64 + r * 8 + 8, :])
                            a0 = _acc(a0, w0 * xr[kt])
                            a1 = _acc(a1, w1 * xr[kt])
                        r0 = (n - MT) * LANE + r * 16
                        qc[r0:r0 + 8, :] = jnp.broadcast_to(_lanesum(a0), (G, LANE))
                        qc[r0 + 8:r0 + 16, :] = jnp.broadcast_to(_lanesum(a1), (G, LANE))
                    tasks_v.append(tv)
            _interleave(tasks_m, tasks_v)
            acc_b[...] = jnp.zeros(acc_b.shape, jnp.float32)

            def qk_body(b, _):
                c0 = b * sb_n
                tasks_m, tasks_v = [], []
                for ci in range(sb_n):
                    for t0 in range(0, MT, NT):
                        def tm(ci=ci, t0=t0):
                            c = c0 + ci
                            g = t0 // NT
                            nt = min(NT, MT - t0)
                            q = _bf(qb[g])
                            kc = _bf(kw[c, t0 * 64:(t0 + nt) * 64, :])
                            for t in range(nt):
                                _row_store(sc, g, c, t, _dot(
                                    q[:, t * LANE:(t + 1) * LANE],
                                    kc[t * LANE:(t + 1) * LANE, :]))
                        tasks_m.append(tm)
                for hv in range(NV):
                    def tv(hv=hv):
                        h = NM + hv
                        qs = [qc[(hv * 24 + j) * 8:(hv * 24 + j + 1) * 8, :]
                              for j in range(24)]
                        for ci in range(sb_n):
                            c = c0 + ci
                            blk = kw[c, h * 96:(h + 1) * 96, :]
                            a0 = a1 = None
                            for d in range(12):
                                k0, k1 = _f32(blk[d * 8:(d + 1) * 8, :])
                                a0 = _acc(a0, k0 * qs[2 * d])
                                a1 = _acc(a1, k1 * qs[2 * d + 1])
                            sc[0, h // G, c, h % G:h % G + 1, :] = jnp.sum(
                                a0 + a1, axis=0, keepdims=True)
                    tasks_v.append(tv)
                _interleave(tasks_m, tasks_v)
                return 0

            jax.lax.fori_loop(0, ns // sb_n, qk_body, 0)

            invs = []
            for g in range(NG):
                n_m = min(max(NM - g * G, 0), G)
                ss = []
                mx = None
                for c in range(ns):
                    s = sc[0, g, c]
                    if n_m:
                        s = s + sc[1, g, c]
                    ss.append(s)
                    mx = s if mx is None else jnp.maximum(mx, s)
                m = jnp.max(mx, axis=1, keepdims=True)
                lsum = None
                for c in range(ns):
                    e = jnp.exp(ss[c] - m)
                    lsum = _acc(lsum, e)
                    if n_m:
                        pb[g, c] = _words(e)
                    if n_m < G:
                        sc[0, g, c] = e
                invs.append(1.0 / _lanesum(lsum))

            def pv_body(b, _):
                c0 = b * sb_n
                tasks_m, tasks_v = [], []
                for ci in range(sb_n):
                    for t0 in range(0, MT, NT):
                        def tm(ci=ci, t0=t0):
                            c = c0 + ci
                            g = t0 // NT
                            nt = min(NT, MT - t0)
                            p = _bf(pb[g, c])
                            vc = _bf(vw[c, t0 * 64:(t0 + nt) * 64, :])
                            for t in range(nt):
                                _row_store(part, g, c, t,
                                           _dot(p, vc[t * LANE:(t + 1) * LANE, :]))
                        tasks_m.append(tm)
                for hv in range(NV):
                    def tv(hv=hv):
                        h = NM + hv
                        ps = [jnp.broadcast_to(
                            sc[0, h // G, c0 + ci, h % G:h % G + 1, :], (G, LANE))
                            for ci in range(sb_n)]
                        for d in range(12):
                            a0 = a1 = None
                            for ci in range(sb_n):
                                v0, v1 = _f32(vw[c0 + ci,
                                                 h * 96 + d * 8:h * 96 + d * 8 + 8, :])
                                a0 = _acc(a0, v0 * ps[ci])
                                a1 = _acc(a1, v1 * ps[ci])
                            r = hv * DH + d * 16
                            acc_b[r:r + 8, :] = acc_b[r:r + 8, :] + a0
                            acc_b[r + 8:r + 16, :] = acc_b[r + 8:r + 16, :] + a1
                    tasks_v.append(tv)
                _interleave(tasks_m, tasks_v)
                return 0

            jax.lax.fori_loop(0, ns // sb_n, pv_body, 0)

            for g in range(MG):
                tot = [None, None]
                for c in range(ns):
                    tot = [_acc(tot[i], part[i, g, c]) for i in range(2)]
                tot = [a * invs[g] for a in tot]
                for t in range(min(NT, MT - g * NT)):
                    ob[g, :, t * LANE:(t + 1) * LANE] = _words(
                        jnp.where(masks[t], tot[1 if t % 3 == 1 else 0], 0.0))

            ys = [None] * ND
            yv = [None] * ND
            tasks_m, tasks_v = [], []
            for kt in range(MT):
                def tm(kt=kt):
                    g, t = divmod(kt, NT)
                    og = _bf(ob[g, :, t * LANE:(t + 1) * LANE])
                    for n in range(ND):
                        ys[n] = _acc(ys[n], _dot(
                            og, _bf(wow[n, kt * 64:(kt + 1) * 64, :]))[0:G])
                tasks_m.append(tm)
            for hv in range(NV):
                def tv(hv=hv):
                    h = NM + hv
                    inv = jnp.broadcast_to(invs[h // G][h % G:h % G + 1, :], (G, LANE))
                    for d in range(12):
                        r = hv * DH + d * 16
                        o0 = _lanesum(acc_b[r:r + 8, :]) * inv
                        o1 = _lanesum(acc_b[r + 8:r + 16, :]) * inv
                        for n in range(ND):
                            w0, w1 = _f32(wow[n, h * 96 + d * 8:h * 96 + d * 8 + 8, :])
                            yv[n] = _acc(yv[n], w0 * o0 + w1 * o1)
                tasks_v.append(tv)
            _interleave(tasks_m, tasks_v)
            x = x + jnp.concatenate(
                [jnp.sum(a + b, axis=0, keepdims=True) for a, b in zip(ys, yv)],
                axis=1)
            return mixer(x, False)

        sc[1] = jnp.zeros(sc.shape[1:], jnp.float32)
        part[...] = jnp.zeros(part.shape, jnp.float32)
        o_ref[...] = layer2(layer1(x0)).astype(o_ref.dtype)

    return kernel


@jax.jit
def pallas_interleave_layers__sliding_block_cached__mixer_s_mlp__decode_kernel(
    A_x: jax.Array,
    A_k_cache: jax.Array,
    A_v_cache: jax.Array,
    A_wq: jax.Array,
    A_wo: jax.Array,
    B_x: jax.Array,
    B_w1: jax.Array,
    B_w2: jax.Array,
    B_w3: jax.Array,
    B_w4: jax.Array,
):
    del B_x, B_w1, B_w2
    sk = A_k_cache.shape[2]
    w = min(4096, max(256, sk // 4))
    ns = w // LANE
    k_t = jnp.transpose(A_k_cache, (0, 1, 3, 2)).reshape(HD, sk)
    v_t = jnp.transpose(A_v_cache, (0, 1, 3, 2)).reshape(HD, sk)
    x2 = A_x.reshape(1, D)

    any_spec = pl.BlockSpec(memory_space=pl.ANY)
    out = pl.pallas_call(
        _make_kernel(sk, w),
        in_specs=[any_spec] * 7,
        out_specs=pl.BlockSpec(memory_space=pltpu.VMEM),
        out_shape=jax.ShapeDtypeStruct((1, D), A_x.dtype),
        scratch_shapes=[
            pltpu.VMEM((1, D), jnp.bfloat16),
            pltpu.VMEM((ns, HD, LANE), jnp.bfloat16),
            pltpu.VMEM((ns, HD, LANE), jnp.bfloat16),
            pltpu.VMEM((HD // LANE, D, LANE), jnp.bfloat16),
            pltpu.VMEM((ND, HD, LANE), jnp.bfloat16),
            pltpu.VMEM((F // LANE, D, LANE), jnp.bfloat16),
            pltpu.VMEM((ND, F, LANE), jnp.bfloat16),
            pltpu.VMEM((NG, G, GR), jnp.int32),
            pltpu.VMEM((2, NG, ns, G, LANE), jnp.float32),
            pltpu.VMEM((NG, ns, G, LANE), jnp.int32),
            pltpu.VMEM((NV * DH, LANE), jnp.float32),
            pltpu.VMEM((NV * DH, LANE), jnp.float32),
            pltpu.VMEM((2, MG, ns, G, LANE), jnp.float32),
            pltpu.VMEM((NG, G, GR), jnp.int32),
            pltpu.SemaphoreType.DMA((2 + W4C,)),
        ],
        compiler_params=pltpu.CompilerParams(
            vmem_limit_bytes=128 * 1024 * 1024),
    )(x2, k_t, v_t, A_wq, A_wo, B_w3, B_w4)
    return out.reshape(A_x.shape)
```
